```python
import os as _os
_os.environ.setdefault("JAX_PLATFORMS", "cpu")
import jax
import jax.numpy as jnp

def _softmax(x, axis=-1):
    return jax.nn.softmax(x, axis=axis)
def _gelu(x):
    return jax.nn.gelu(x, approximate=True)
def _silu(x):
    return jax.nn.silu(x)
def _sigmoid(x):
    return jax.nn.sigmoid(x)
def _layernorm(x, axis=-1, eps=1e-5):
    m = jnp.mean(x, axis=axis, keepdims=True)
    v = jnp.var(x, axis=axis, keepdims=True)
    return (x - m) / jnp.sqrt(v + eps)
def _scatter_add(tgt, idx, src, axis=0):
    return tgt.at[idx].add(src)
def _segment_sum(src, seg, n):
    return jax.ops.segment_sum(src, seg, n)
class _Rng:
    def __init__(self, key):
        self._k = key
    def _next(self):
        self._k, sub = jax.random.split(self._k)
        return sub
    def normal(self, shape):
        return jax.random.normal(self._next(), shape, dtype=jnp.bfloat16)
    def randint(self, lo, hi, shape):
        return jax.random.randint(self._next(), shape, lo, hi, dtype=jnp.int32)
    def uniform(self, shape, lo=0.0, hi=1.0):
        return jax.random.uniform(self._next(), shape, jnp.bfloat16, lo, hi)
    def permutation(self, n):
        return jax.random.permutation(self._next(), n)


kernel_name = 'concat_heads__gqa_block_cached__mha_block_cached__near_ridge'

def setup_inputs():
    _rng = _Rng(jax.random.key(int.from_bytes(__import__("os").urandom(4), "little")))
    _w = (lambda a: (lambda t: t.astype(jnp.bfloat16) if jnp.issubdtype(t.dtype, jnp.floating) else t)(jnp.asarray(a)))
    def _A_setup():
        B, Sq, D = 8, 48, 512
        Hq, Hkv, Sk, Dh = 32, 8, 1024, 128
        assert Hq % Hkv == 0, (Hq, Hkv)
        return {
            "x": _w((lambda *s: _rng.normal(s) * 0.8)(B, Sq, D)),
            "k_cache": _w((lambda *s: _rng.normal(s) * 0.8)(B, Hkv, Sk, Dh)),
            "v_cache": _w((lambda *s: _rng.normal(s) * 0.05)(B, Hkv, Sk, Dh)),
            "wq": _w((lambda *s: _rng.normal(s) * 0.8)(D, Hq * Dh) * (D ** -0.5)),
            "wo": _w((lambda *s: _rng.normal(s) * 0.05)(Hq * Dh, D) * ((Hq * Dh) ** -0.5)),
        }
    _A_in = _A_setup()

    def _B_setup():
        B, Sq, D = 8, 48, 512
        H, Sk, Dh = 32, 1024, 128
        return {
            "x": _w((lambda *s: _rng.normal(s) * 0.8)(B, Sq, D)),
            "k_cache": _w((lambda *s: _rng.normal(s) * 0.8)(B, H, Sk, Dh)),
            "v_cache": _w((lambda *s: _rng.normal(s) * 0.05)(B, H, Sk, Dh)),
            "wq": _w((lambda *s: _rng.normal(s) * 0.8)(D, H * Dh) * (D ** -0.5)),
            "wo": _w((lambda *s: _rng.normal(s) * 0.05)(H * Dh, D) * ((H * Dh) ** -0.5)),
        }
    _B_in = _B_setup()

    return {
        "A_x": _A_in["x"],
        "A_k_cache": _A_in["k_cache"],
        "A_v_cache": _A_in["v_cache"],
        "A_wq": _A_in["wq"],
        "A_wo": _A_in["wo"],
        "B_x": _B_in["x"],
        "B_k_cache": _B_in["k_cache"],
        "B_v_cache": _B_in["v_cache"],
        "B_wq": _B_in["wq"],
        "B_wo": _B_in["wo"],
    }

def reference(A_x, A_k_cache, A_v_cache, A_wq, A_wo, B_x, B_k_cache, B_v_cache, B_wq, B_wo):
    def _A_ref(x, k_cache, v_cache, wq, wo):
        B, Sq, D = x.shape
        Hq, Dh = 32, 128
        Hkv = k_cache.shape[1]
        rep = Hq // Hkv
        q = (lambda x, *d: x.transpose(*d))((x @ wq).reshape(B, Sq, Hq, Dh), 0, 2, 1, 3)
        k = jnp.repeat(k_cache, rep, axis=1)
        v = jnp.repeat(v_cache, rep, axis=1)
        scores = jnp.einsum("bhqd,bhkd->bhqk", q, k) * (Dh ** -0.5)
        p = _softmax(scores, axis=-1)
        o = jnp.einsum("bhqk,bhkd->bhqd", p, v)
        return (lambda x, *d: x.transpose(*d))(o, 0, 2, 1, 3).reshape(B, Sq, Hq * Dh) @ wo

    def _B_ref(x, k_cache, v_cache, wq, wo):
        B, Sq, D = x.shape
        H, Dh = 32, 128
        q = (lambda x, *d: x.transpose(*d))((x @ wq).reshape(B, Sq, H, Dh), 0, 2, 1, 3)
        scores = jnp.einsum("bhqd,bhkd->bhqk", q, k_cache) * (Dh ** -0.5)
        p = _softmax(scores, axis=-1)
        o = jnp.einsum("bhqk,bhkd->bhqd", p, v_cache)
        return (lambda x, *d: x.transpose(*d))(o, 0, 2, 1, 3).reshape(B, Sq, H * Dh) @ wo

    a = _A_ref(A_x, A_k_cache, A_v_cache, A_wq, A_wo)
    b = _B_ref(B_x, B_k_cache, B_v_cache, B_wq, B_wo)
    return jnp.concatenate([a, b], axis=-1)
```

```python
import functools
import math

import jax
import jax.numpy as jnp
import jax.experimental.pallas as pl
import jax.experimental.pallas.tpu as pltpu

NB, SQ, D = 8, 48, 512
H, HKV, SK, DH = 32, 8, 1024, 128
M = NB * SQ
G = 8
BLK = 256
QSCALE = (DH ** -0.5) * math.log2(math.e)


def attn(q, k, v):
    s = jax.lax.dot_general(q, k, (((1,), (1,)), ((), ())), preferred_element_type=jnp.float32)
    m = jnp.max(s, axis=-1, keepdims=True)
    p = jnp.exp2(s - m)
    l = jnp.sum(p, axis=-1, keepdims=True)
    o = jnp.dot(p.astype(jnp.bfloat16), v, preferred_element_type=jnp.float32)
    return (o * (1.0 / l)).astype(jnp.bfloat16)


def build(mode="split", small=16, compute=True, nslot=3, npoints=5, name="attn_v1", order="r5", dma=True,
          nobounds=True):
    look = 2

    blocks = []
    if order == "r5":
        for r in range(8):
            sl, j = r // 4, r % 4
            blocks += [(2 + sl, j), (6 + sl, j), (4 + sl, j), (8 + sl, j), (r % 2, r // 2)]
    elif order == "seq":
        blocks = [(sl, j) for sl in range(10) for j in range(4)]
    assert sorted(blocks) == [(sl, j) for sl in range(10) for j in range(4)]

    def kernel(xa, ka, va, wqa, woa, xb, kb, vb, wqb, wob, out,
               kv_buf, x_buf, wq_buf, wo_buf, q_buf, o_buf, acc, out_buf,
               kv_sem, x_sem, wq_sem, wo_sem, out_sem):
        wq_hbm = (wqa, wqb)
        wo_hbm = (woa, wob)

        def kv_copy(g, b, slot, slab, r0, nr):
            if slab == 0:
                src = ka.at[b, g]
            elif slab == 1:
                src = va.at[b, g]
            elif slab < 6:
                src = kb.at[b, 4 * g + (slab - 2)]
            else:
                src = vb.at[b, 4 * g + (slab - 6)]
            return pltpu.make_async_copy(src.at[pl.ds(r0, nr)], kv_buf.at[slot, slab, pl.ds(r0, nr)], kv_sem.at[slot])

        def wq_copy(br, g, r0, nr):
            c0 = g * 512 if isinstance(g, int) else pl.multiple_of(g * 512, 512)
            return pltpu.make_async_copy(wq_hbm[br].at[pl.ds(r0, nr), pl.ds(c0, 512)],
                                         wq_buf.at[g, br, pl.ds(r0, nr)], wq_sem.at[g])

        def wo_copy(br, g, r0, nr):
            return pltpu.make_async_copy(wo_hbm[br].at[pl.ds(g * 512 + r0, nr)],
                                         wo_buf.at[g, br, pl.ds(r0, nr)], wo_sem.at[g])

        def issue_list(g, b, slot, with_wq, with_wo):
            ops = []
            r0 = b * 64 if isinstance(b, int) else pl.multiple_of(b * 64, 64)
            if mode == "split":
                w = []
                if with_wq:
                    w += [lambda br=br: wq_copy(br, g + 2, r0, 64).start(priority=1) for br in (0, 1)]
                if with_wo:
                    w += [lambda br=br: wo_copy(br, g, r0, 64).start(priority=1) for br in (0, 1)]
                for i, (slab, j) in enumerate(blocks):
                    big = BLK - small
                    ops.append(lambda slab=slab, j=j: kv_copy(g, b, slot, slab, j * BLK, big).start(priority=1))
                    if small:
                        ops.append(lambda slab=slab, j=j: kv_copy(g, b, slot, slab, j * BLK + big, small).start(priority=0))
                    if i % 10 == 9 and w:
                        ops.append(w.pop(0))
                assert not w
            elif mode == "wfill":
                w = []
                for i in range(8):
                    for br in (0, 1):
                        if with_wq:
                            w.append(lambda br=br, i=i: wq_copy(br, g + 2, r0 + 8 * i, 8).start(priority=0))
                        if with_wo:
                            w.append(lambda br=br, i=i: wo_copy(br, g, r0 + 8 * i, 8).start(priority=0))
                nw = len(w)
                for i, (slab, j) in enumerate(blocks):
                    if nw == 32 or (nw == 16 and i % 5 in (0, 2)):
                        ops.append(lambda slab=slab, j=j: kv_copy(g, b, slot, slab, j * BLK, BLK).start(priority=1))
                        if w and (nw == 16 or i % 5 != 4):
                            ops.append(w.pop(0))
                    else:
                        big = BLK - small
                        ops.append(lambda slab=slab, j=j: kv_copy(g, b, slot, slab, j * BLK, big).start(priority=1))
                        ops.append(lambda slab=slab, j=j: kv_copy(g, b, slot, slab, j * BLK + big, small).start(priority=0))
                assert not w
            elif mode == "plain":
                for slab in range(10):
                    ops.append(lambda slab=slab: kv_copy(g, b, slot, slab, 0, SK).start())
                if with_wq:
                    ops += [lambda br=br: wq_copy(br, g + 2, r0, 64).start() for br in (0, 1)]
                if with_wo:
                    ops += [lambda br=br: wo_copy(br, g, r0, 64).start() for br in (0, 1)]
            if not dma:
                ops = []
            return ops

        def wait_kv(slot):
            if dma:
                pltpu.make_async_copy(kv_buf.at[slot], kv_buf.at[slot], kv_sem.at[slot]).wait()

        def wait_wq(g):
            if dma:
                pltpu.make_async_copy(wq_buf.at[g], wq_buf.at[g], wq_sem.at[g]).wait()

        def wait_wo(g):
            if dma:
                pltpu.make_async_copy(wo_buf.at[g], wo_buf.at[g], wo_sem.at[g]).wait()

        def q_proj(g, j):
            br = j // 4
            c0 = (j % 4) * DH
            if not isinstance(j, int):
                c0 = pl.multiple_of(c0, DH)
            w = wq_buf[g, br, :, pl.ds(c0, DH)]
            q = jnp.dot(x_buf[br], w, preferred_element_type=jnp.float32)
            q_buf[g % 2, j] = (q * QSCALE).astype(jnp.bfloat16)

        def o_proj(g, j):
            br = j // 4
            c0 = (j % 4) * DH
            if not isinstance(j, int):
                c0 = pl.multiple_of(c0, DH)
            w = wo_buf[g, br, :, pl.ds(c0, DH)]
            return jnp.dot(o_buf[g % 2, br], w, preferred_element_type=jnp.float32)

        def step(g, b, slot, ops, do_q, do_o):
            n = len(ops)
            cuts = [n * i // npoints for i in range(npoints + 1)]
            parts = [ops[cuts[i]:cuts[i + 1]] for i in range(npoints)]

            def issue(i):
                if i < npoints:
                    for f in parts[i]:
                        f()

            rows = pl.ds(pl.multiple_of(b * SQ, SQ), SQ)
            par = g % 2
            issue(0)
            if compute:
                qa = jnp.concatenate([q_buf[par, j, rows, :] for j in range(4)], axis=0)
                oa = attn(qa, kv_buf[slot, 0], kv_buf[slot, 1])
                for j in range(4):
                    o_buf[par, 0, rows, j * DH:(j + 1) * DH] = oa[j * SQ:(j + 1) * SQ]
            for j in range(4):
                issue(1 + j)
                if compute:
                    ob = attn(q_buf[par, 4 + j, rows, :], kv_buf[slot, 2 + j], kv_buf[slot, 6 + j])
                    o_buf[par, 1, rows, j * DH:(j + 1) * DH] = ob
            if compute:
                if do_q:
                    q_proj(g + 1, b)
                if do_o:
                    acc[b] += o_proj(g - 1, b)

        if dma:
            xc = [pltpu.make_async_copy(xa, x_buf.at[0], x_sem.at[0]), pltpu.make_async_copy(xb, x_buf.at[1], x_sem.at[1])]
            for c in xc:
                c.start(priority=1)
            for i in range(8):
                for br in (0, 1):
                    wq_copy(br, 0, 64 * i, 64).start(priority=1)
        for f in issue_list(0, 0, 0, True, True):
            f()
        if dma:
            for i in range(8):
                for br in (0, 1):
                    wq_copy(br, 1, 64 * i, 64).start(priority=1)
            for c in xc:
                c.wait()
        wait_wq(0)
        ops1 = issue_list(0, 1, 1, True, True)
        for j in range(8):
            for f in ops1[len(ops1) * j // 8: len(ops1) * (j + 1) // 8]:
                f()
            if compute:
                q_proj(0, j)
        acc[...] = jnp.zeros_like(acc)

        def run(s_lo, s_hi, with_wq, with_wo, do_issue, do_q, do_o):
            def body(s, c):
                g, b = s // 8, s % 8
                slot = s % nslot
                t = s + look

                @pl.when(b == 0)
                def _():
                    if do_q:
                        wait_wq(g + 1)
                    if do_o:
                        wait_wo(g - 1)

                wait_kv(slot)
                ops = issue_list(t // 8, t % 8, t % nslot, with_wq, with_wo) if do_issue else []
                step(g, b, slot, ops, do_q, do_o)
                return c
            jax.lax.fori_loop(s_lo, s_hi, body, 0)

        run(0, 8, True, True, True, True, False)
        run(8, 46, True, True, True, True, True)
        run(46, 56, False, True, True, True, True)
        run(56, 62, False, True, True, False, True)
        run(62, 64, False, False, False, False, True)

        wait_wo(7)
        for j in range(8):
            if compute:
                r = acc[j] + o_proj(7, j)
            else:
                r = acc[j]
            out_buf[:, j * DH:(j + 1) * DH] = r.astype(jnp.bfloat16)
        oc = pltpu.make_async_copy(out_buf, out, out_sem)
        oc.start()
        oc.wait()

    def fn(A_x, A_k, A_v, A_wq, A_wo, B_x, B_k, B_v, B_wq, B_wo):
        bf = jnp.bfloat16
        out = pl.pallas_call(
            kernel,
            in_specs=[pl.BlockSpec(memory_space=pltpu.HBM)] * 10,
            out_specs=pl.BlockSpec(memory_space=pltpu.HBM),
            out_shape=jax.ShapeDtypeStruct((M, 2 * D), bf),
            scratch_shapes=[
                pltpu.VMEM((nslot, 10, SK, DH), bf),
                pltpu.VMEM((2, M, D), bf),
                pltpu.VMEM((G, 2, D, 512), bf),
                pltpu.VMEM((G, 2, 512, D), bf),
                pltpu.VMEM((2, 8, M, DH), bf),
                pltpu.VMEM((2, 2, M, 512), bf),
                pltpu.VMEM((8, M, DH), jnp.float32),
                pltpu.VMEM((M, 2 * D), bf),
                pltpu.SemaphoreType.DMA((nslot,)),
                pltpu.SemaphoreType.DMA((2,)),
                pltpu.SemaphoreType.DMA((G,)),
                pltpu.SemaphoreType.DMA((G,)),
                pltpu.SemaphoreType.DMA,
            ],
            compiler_params=pltpu.CompilerParams(vmem_limit_bytes=100 * 2**20, disable_bounds_checks=nobounds),
            name=name,
        )(A_x.reshape(M, D), A_k, A_v, A_wq, A_wo, B_x.reshape(M, D), B_k, B_v, B_wq, B_wo)
        return out.reshape(NB, SQ, 2 * D)
    return fn


@jax.jit
def pallas_concat_heads__gqa_block_cached__mha_block_cached__near_ridge_kernel(
    A_x, A_k_cache, A_v_cache, A_wq, A_wo, B_x, B_k_cache, B_v_cache, B_wq, B_wo):
    return build()(A_x, A_k_cache, A_v_cache, A_wq, A_wo, B_x, B_k_cache, B_v_cache, B_wq, B_wo)
```

```python
import math

import jax
import jax.numpy as jnp
import jax.experimental.pallas as pl
import jax.experimental.pallas.tpu as pltpu

NB, SQ, D = 8, 48, 512
H, HKV, SK, DH = 32, 8, 1024, 128
M = NB * SQ
G = 8
QSCALE = (DH ** -0.5) * math.log2(math.e)
NS = 3
f32, bf16 = jnp.float32, jnp.bfloat16


def qk(q, k):
    return jax.lax.dot_general(q, k, (((1,), (1,)), ((), ())), preferred_element_type=f32)


def softmax_parts(s):
    m = jnp.max(s, axis=-1, keepdims=True)
    p = jnp.exp2(s - m)
    l = jnp.sum(p, axis=-1, keepdims=True)
    return p.astype(bf16), l


def pv(p, l, v):
    o = jnp.dot(p, v, preferred_element_type=f32)
    return (o * (1.0 / l)).astype(bf16)


def merge(*lists, phase=None):
    m = []
    for w, l in enumerate(lists):
        ph = 0.5 if phase is None else phase[w]
        m += [((i + ph) / len(l), w, i) for i in range(len(l))]
    m.sort()
    return [lists[w][i] for _, w, i in m]


def mo(x, n):
    return x if isinstance(x, int) else pl.multiple_of(x, n)


def build(name="attn_v2", compute=True, dma=True, ysplit=640, head=128, hsm=32, npoints=8, nobounds=True,
          final_groups=((0, 4), (4, 2), (6, 1), (7, 1)), out_prio=0, skew=2, nosem=False):
    def kernel(xa, ka, va, wqa, woa, xb, kb, vb, wqb, wob, out,
               kvb, kva, ka0, x_buf, wq_buf, wo_buf, acc_a, acc_b, out_buf,
               sems, out_sem):
        wq_hbm, wo_hbm = (wqa, wqb), (woa, wob)
        ctx = {}
        kv_sem = lambda slot: sems.at[slot + ctx["z"]]
        a0_sem = lambda p: sems.at[NS + p + ctx["z"]]
        x_sem = lambda: sems.at[NS + 2 + ctx["z"]]
        w_sem = lambda g: sems.at[NS + 3 + g + ctx["z"]]
        fin_sem = lambda i: sems.at[NS + 3 + G + i + ctx["z"]]

        def b_copy(h, slot, a, b0, nb, r0, nr, sem=None):
            src = (kb, vb)[a].at[pl.ds(b0, nb), h, pl.ds(r0, nr)]
            dst = kvb.at[slot, a, pl.ds(b0, nb), pl.ds(r0, nr)]
            return pltpu.make_async_copy(src, dst, kv_sem(slot) if sem is None else fin_sem(sem))

        def a_copy(p, slot, a, b0, nb, r0, nr):
            src = (ka, va)[a].at[pl.ds(2 * (p % 4) + b0, nb), p // 4, pl.ds(r0, nr)]
            if isinstance(p, int) and p < 2:
                dst, sem = ka0.at[p, a, pl.ds(b0, nb), pl.ds(r0, nr)], a0_sem(p)
            else:
                dst, sem = kva.at[slot, a, pl.ds(b0, nb), pl.ds(r0, nr)], kv_sem(slot)
            return pltpu.make_async_copy(src, dst, sem)

        def wq_copy(br, g, r0, nr):
            return pltpu.make_async_copy(wq_hbm[br].at[pl.ds(r0, nr), pl.ds(mo(g * 512, 512), 512)],
                                         wq_buf.at[br, g, pl.ds(r0, nr)], w_sem(g))

        def wo_copy(br, g, r0, nr):
            return pltpu.make_async_copy(wo_hbm[br].at[pl.ds(mo(g * 512 + r0, 8), nr)],
                                         wo_buf.at[br, g, pl.ds(r0, nr)], w_sem(g))

        def start(mk, prio, *args, **kw):
            return lambda: mk(*args, **kw).start(priority=prio)

        def kv_main(t, slot, lo, hi, with_a=True):
            bs = [start(b_copy, 1, t, slot, a, b0, 4, r0, 64) for r0 in range(lo, hi, 64) for b0 in (0, 4) for a in (0, 1)]
            if not with_a:
                return bs
            as_ = [start(a_copy, 1, t + 2, slot, a, 0, 2, r0, 128) for r0 in range(lo, hi, 128) for a in (0, 1)]
            return merge(bs, as_)

        def kv_fill(t, slot, with_a=True):
            bs = [start(b_copy, 0, t, slot, a, b, 1, r0, hsm) for r0 in range(0, head, hsm) for b in range(8) for a in (0, 1)]
            if not with_a:
                return bs
            as_ = [start(a_copy, 0, t + 2, slot, a, b, 1, r0, hsm) for r0 in range(0, head, hsm) for b in range(2) for a in (0, 1)]
            return merge(bs, as_)

        def w_fill(g, j):
            qs = [start(wq_copy, 0, br, g, mo(64 * i + 16 * j + k, 8), 8) for k in (0, 8) for i in range(8) for br in (0, 1)]
            os_ = [start(wo_copy, 0, br, g, mo(128 * j + r0, 8), 8) for r0 in range(0, 128, 8) for br in (0, 1)]
            return merge(qs, os_)

        def x_fill():
            return [start(lambda br, r0: pltpu.make_async_copy((xa, xb)[br].at[pl.ds(r0, 8)], x_buf.at[br, pl.ds(r0, 8)], x_sem()), 0, br, r0)
                    for r0 in range(0, M, 8) for br in (0, 1)]

        def fin_ops():
            ops = []
            slot = 31 % NS
            for gi, (b0, nb) in enumerate(final_groups):
                if nb > 1:
                    r = 256 // nb
                    t1 = [start(b_copy, 1, 31, slot, a, b0, nb, r0, r, 2 * gi + a) for r0 in range(head, SK, r) for a in (0, 1)]
                    t0 = [start(b_copy, 0, 31, slot, a, b, 1, r0, hsm, 2 * gi + a)
                          for r0 in range(0, head, hsm) for b in range(b0, b0 + nb) for a in (0, 1)]
                    ops += merge(t1, t0, phase=(0.5, 0.25))
                else:
                    for a in (0, 1):
                        for r0 in range(0, SK, 256):
                            ops.append(start(b_copy, 0, 31, slot, a, b0, 1, r0, 16, 2 * gi + a))
                            ops.append(start(b_copy, 1, 31, slot, a, b0, 1, r0 + 16, 240, 2 * gi + a))
            return ops

        def window(s, kind):
            s1 = (s + 1) % NS
            s2 = (s + 2) % NS
            if kind == "W":
                t1 = kv_main(s + 1, s1, ysplit, SK) + kv_main(s + 2, s2, 0, ysplit)
                t0 = w_fill(s // 4 + 2, s % 4)
            elif kind == "T":
                t1 = kv_main(s + 1, s1, ysplit, SK) + kv_main(s + 2, s2, head, ysplit)
                t0 = kv_fill(s + 2, s2)
            elif kind == "T28":
                t1 = kv_main(s + 1, s1, ysplit, SK) + kv_main(s + 2, s2, head, ysplit, with_a=False)
                t0 = kv_fill(s + 2, s2, with_a=False)
            return merge(t1, t0, phase=(0.5, 0.75))

        def wait_step(slot, with_a=True):
            if dma:
                pltpu.make_async_copy(kvb.at[slot], kvb.at[slot], kv_sem(slot)).wait()
                if with_a:
                    pltpu.make_async_copy(kva.at[slot], kva.at[slot], kv_sem(slot)).wait()

        def wait_w(g):
            if dma:
                pltpu.make_async_copy(wq_buf.at[:, g], wq_buf.at[:, g], w_sem(g)).wait()
                pltpu.make_async_copy(wo_buf.at[:, g], wo_buf.at[:, g], w_sem(g)).wait()

        def a_rows(p):
            return pl.ds(mo((p % 4) * 2 * SQ, 2 * SQ), 2 * SQ)

        def a_qproj(p):
            q = jnp.dot(x_buf[0, a_rows(p), :], wq_buf[0, p // 4], preferred_element_type=f32)
            q = (q * QSCALE).astype(bf16)
            return [jnp.concatenate([q[u * SQ:(u + 1) * SQ, i * DH:(i + 1) * DH] for i in range(4)], axis=0) for u in range(2)]

        def a_oproj(p, o, first=False, last=False):
            o = jnp.concatenate([jnp.concatenate([o[u][i * SQ:(i + 1) * SQ] for i in range(4)], axis=1) for u in range(2)], axis=0)
            r = jnp.dot(o, wo_buf[0, p // 4], preferred_element_type=f32)
            if not first:
                r = r + acc_a[a_rows(p), :]
            if last:
                out_buf[a_rows(p), 0:D] = r.astype(bf16)
            else:
                acc_a[a_rows(p), :] = r

        def b_qproj(h):
            w = wq_buf[1, h // 4, :, pl.ds(mo((h % 4) * DH, DH), DH)]
            q = jnp.dot(x_buf[1], w, preferred_element_type=f32)
            return (q * QSCALE).astype(bf16)

        def b_oproj(h, o, b0, last=False):
            w = wo_buf[1, h // 4, pl.ds(mo((h % 4) * DH, DH), DH), :]
            rows = pl.ds(b0 * SQ, len(o) * SQ)
            o = o[0] if len(o) == 1 else jnp.concatenate(o, axis=0)
            r = jnp.dot(o, w, preferred_element_type=f32) + acc_b[rows, :]
            if last:
                out_buf[rows, D:2 * D] = r.astype(bf16)
            else:
                acc_b[rows, :] = r

        def run_tasks(tasks, ops):
            if not dma:
                ops = []
            if not compute:
                for f in ops:
                    f()
                return
            total = sum(w for w, _ in tasks)
            pos, done, point = 0.0, 0, 0
            for w, fn in tasks:
                if point < npoints and pos >= total * point / npoints - 1e-9:
                    while point < npoints and pos >= total * point / npoints - 1e-9:
                        point += 1
                    upto = len(ops) * point // npoints
                    for f in ops[done:upto]:
                        f()
                    done = upto
                fn()
                pos += w
            for f in ops[done:]:
                f()

        def step_tasks(s, slot, with_a=True, with_b=True, a_first=False, a_last=False, a_src=None):
            st = {}
            T = []
            p = s + 2
            ak = (lambda u, a: kva[slot, a, u]) if a_src is None else a_src
            units = ([("a", 0), ("a", 1)] if with_a else []) + ([("b", b) for b in range(NB)] if with_b else [])
            if with_a:
                T.append((384, lambda: st.__setitem__("qa", a_qproj(p))))
            if with_b:
                T.append((384, lambda: st.__setitem__("qb", b_qproj(s))))

            def do_qk(kind, u):
                if kind == "a":
                    st["s", kind, u] = qk(st["qa"][u], ak(u, 0))
                else:
                    st["s", kind, u] = qk(st["qb"][u * SQ:(u + 1) * SQ], kvb[slot, 0, u])

            def do_pv(kind, u):
                v = ak(u, 1) if kind == "a" else kvb[slot, 1, u]
                st["o", kind, u] = pv(*softmax_parts(st.pop(("s", kind, u))), v)

            sk = skew if with_b else 1
            for t in range(len(units) + sk):
                if t < len(units):
                    T.append((400 if units[t][0] == "a" else 128, lambda x=units[t]: do_qk(*x)))
                if t - sk >= 0:
                    x = units[t - sk]
                    T.append((400 if x[0] == "a" else 110, lambda x=x: do_pv(*x)))
                    if with_a and with_b and x == ("b", 1):
                        T.append((384, lambda: a_oproj(p, [st.pop(("o", "a", u)) for u in range(2)], a_first, a_last)))
                    if x == ("b", 5):
                        T.append((192, lambda: b_oproj(s, [st.pop(("o", "b", u)) for u in range(4)], 0)))
            if with_a and not with_b:
                T.append((384, lambda: a_oproj(p, [st.pop(("o", "a", u)) for u in range(2)], a_first, a_last)))
            if with_b:
                T.append((192, lambda: b_oproj(s, [st.pop(("o", "b", u)) for u in range(4, 8)], 4)))
            return T

        def out_copy(r0, nr, c0, i):
            return pltpu.make_async_copy(out_buf.at[pl.ds(r0, nr), pl.ds(c0, D)], out.at[pl.ds(r0, nr), pl.ds(c0, D)], out_sem.at[i])

        def prologue():
            a_pre = [[start(a_copy, 1, p, 0, a, 0, 2, r0, 128) for r0 in range(0, SK, 128) for a in (0, 1)] for p in range(2)]
            w0 = [f for j in range(4) for f in w_fill(0, j)]
            w1 = [f for j in range(4) for f in w_fill(1, j)]
            pro_t1 = a_pre[0] + a_pre[1] + kv_main(0, 0, 0, SK) + kv_main(1, 1, 0, ysplit)
            pro_t0 = merge(x_fill(), w0) + w1
            pro = merge(pro_t1, pro_t0, phase=(0.5, 0.5))
            n_first = (len(pro) * (len(pro_t0) - len(w1))) // len(pro_t0) + 2
            if dma:
                for f in pro[:n_first]:
                    f()
            acc_a[...] = jnp.zeros_like(acc_a)
            acc_b[...] = jnp.zeros_like(acc_b)
            if dma:
                pltpu.make_async_copy(x_buf, x_buf, x_sem()).wait()
            wait_w(0)
            rest = pro[n_first:]
            for p in range(2):
                if dma:
                    pltpu.make_async_copy(ka0.at[p], ka0.at[p], a0_sem(p)).wait()
                run_tasks(step_tasks(p - 2, 0, with_b=False, a_src=lambda u, a, p=p: ka0[p, a, u]),
                          rest[len(rest) * p // 2: len(rest) * (p + 1) // 2])

        def full_step(s, kind):
            wait_step(s % NS)
            run_tasks(step_tasks(s, s % NS), window(s, kind))

        def step29(s):
            fin = fin_ops()
            ny = len(fin) * ysplit // SK
            x30 = kv_main(30, 30 % NS, ysplit, SK, with_a=False)
            wait_step(29 % NS)
            run_tasks(step_tasks(29, 29 % NS), x30 + fin[:ny])
            out_buf[:, 0:D] = acc_a[...].astype(bf16)
            out_copy(0, M, 0, 0).start(priority=out_prio)

        def step30(s):
            fin = fin_ops()
            ny = len(fin) * ysplit // SK
            wait_step(30 % NS, with_a=False)
            run_tasks(step_tasks(30, 30 % NS, with_a=False), fin[ny:])
            slot = 31 % NS
            outs = [out_copy(0, M, 0, 0)]
            qb = b_qproj(31) if compute else None
            for gi, (b0, nb) in enumerate(final_groups):
                def w(a):
                    if dma:
                        r = kvb.at[slot, a, pl.ds(b0, nb)]
                        pltpu.make_async_copy(r, r, fin_sem(2 * gi + a)).wait()
                w(0)
                if nb > 1:
                    w(1)
                if compute:
                    ss = [qk(qb[u * SQ:(u + 1) * SQ], kvb[slot, 0, u]) for u in range(b0, b0 + nb)]
                    ps = [softmax_parts(x) for x in ss]
                if nb == 1:
                    w(1)
                if compute:
                    os_ = [pv(*ps[i], kvb[slot, 1, b0 + i]) for i in range(nb)]
                    b_oproj(31, os_, b0, last=True)
                else:
                    out_buf[pl.ds(b0 * SQ, nb * SQ), D:2 * D] = acc_b[pl.ds(b0 * SQ, nb * SQ), :].astype(bf16)
                oc = out_copy(b0 * SQ, nb * SQ, D, 1 + gi)
                oc.start(priority=out_prio)
                outs.append(oc)
            for oc in outs:
                oc.wait()

        def body(i, c):
            s = i - 1

            @pl.when(i == 0)
            def _():
                ctx["z"] = i
                prologue()

            @pl.when(jnp.logical_and(s >= 0, s < 30))
            def _():
                ctx["z"] = 0

                @pl.when(jnp.logical_and(s % 4 == 2, s < 28))
                def _():
                    wait_w((s + 2) // 4)

            @pl.when(jnp.logical_and(s >= 0, s < 24))
            def _():
                ctx["z"] = 0
                full_step(s, "W")

            @pl.when(jnp.logical_and(s >= 24, s < 28))
            def _():
                ctx["z"] = 0
                full_step(s, "T")

            @pl.when(s == 28)
            def _():
                ctx["z"] = s - 28
                full_step(28, "T28")

            @pl.when(s == 29)
            def _():
                ctx["z"] = s - 29
                step29(s)

            @pl.when(s == 30)
            def _():
                ctx["z"] = s - 30
                step30(s)
            return c

        jax.lax.fori_loop(0, 32, body, 0)

    def fn(A_x, A_k, A_v, A_wq, A_wo, B_x, B_k, B_v, B_wq, B_wo):
        nf = len(final_groups)
        out = pl.pallas_call(
            kernel,
            in_specs=[pl.BlockSpec(memory_space=pltpu.HBM)] * 10,
            out_specs=pl.BlockSpec(memory_space=pltpu.HBM),
            out_shape=jax.ShapeDtypeStruct((M, 2 * D), bf16),
            scratch_shapes=[
                pltpu.VMEM((NS, 2, NB, SK, DH), bf16),
                pltpu.VMEM((NS, 2, 2, SK, DH), bf16),
                pltpu.VMEM((2, 2, 2, SK, DH), bf16),
                pltpu.VMEM((2, M, D), bf16),
                pltpu.VMEM((2, G, D, 512), bf16),
                pltpu.VMEM((2, G, 512, D), bf16),
                pltpu.VMEM((M, D), f32),
                pltpu.VMEM((M, D), f32),
                pltpu.VMEM((M, 2 * D), bf16),
                pltpu.SemaphoreType.DMA((NS + 3 + G + 2 * nf,)),
                pltpu.SemaphoreType.DMA((1 + nf,)),
            ],
            compiler_params=pltpu.CompilerParams(vmem_limit_bytes=100 * 2**20, disable_bounds_checks=nobounds,
                                                 disable_semaphore_checks=nosem),
            name=name,
        )(A_x.reshape(M, D), A_k, A_v, A_wq, A_wo, B_x.reshape(M, D), B_k, B_v, B_wq, B_wo)
        return out.reshape(NB, SQ, 2 * D)
    return fn


@jax.jit
def pallas_concat_heads__gqa_block_cached__mha_block_cached__near_ridge_kernel(
    A_x, A_k_cache, A_v_cache, A_wq, A_wo, B_x, B_k_cache, B_v_cache, B_wq, B_wo):
    return build()(A_x, A_k_cache, A_v_cache, A_wq, A_wo, B_x, B_k_cache, B_v_cache, B_wq, B_wo)
```

```python
import math

import jax
import jax.numpy as jnp
import jax.experimental.pallas as pl
import jax.experimental.pallas.tpu as pltpu

NB, SQ, D = 8, 48, 512
H, HKV, SK, DH = 32, 8, 1024, 128
M = NB * SQ
G = 8
QSCALE = (DH ** -0.5) * math.log2(math.e)
f32, bf16 = jnp.float32, jnp.bfloat16


def qk(q, k):
    return jax.lax.dot_general(q, k, (((1,), (1,)), ((), ())), preferred_element_type=f32)


def softmax_parts(s):
    m = jnp.max(s, axis=-1, keepdims=True)
    p = jnp.exp2(s - m)
    l = jnp.sum(p, axis=-1, keepdims=True)
    return p.astype(bf16), l


def pv(p, l, v):
    o = jnp.dot(p, v, preferred_element_type=f32)
    return (o * (1.0 / l)).astype(bf16)


def merge(*lists, phase=None):
    m = []
    for w, l in enumerate(lists):
        ph = 0.5 if phase is None else phase[w]
        m += [((i + ph) / len(l), w, i) for i in range(len(l))]
    m.sort()
    return [lists[w][i] for _, w, i in m]


def mo(x, n):
    return x if isinstance(x, int) else pl.multiple_of(x, n)


def build(name="attn_v5", compute=True, dma=True, ysplit=832, head=192, hsm=64, npoints=4, nobounds=True, nosem=True,
          skew=2, vcut=768, lead=27, fine=0, fhead=128, fhsm=32, pvsplit=True, pro_mode=0, xfill=True, wr_rows=False, cmask=7, afrac=0.25):
    compute0 = compute

    def kernel(xa, ka, va, wqa, woa, xb, kb, vb, wqb, wob, out,
               kv_buf, x_buf, w_buf, acc_a, acc_b, out_buf, sems, out_sem):
        ctx = {"z": 0}
        kv_sem = lambda g, slot: sems.at[5 * (g % 2) + slot + ctx["z"]]
        w_sem = lambda g: sems.at[10 + g + ctx["z"]]
        fin_sem = lambda i: sems.at[10 + G + i + ctx["z"]]

        def kv_copy(g, slot, a, b0, nb, r0, nr, fin=None):
            if slot == 4:
                src = (ka, va)[a].at[pl.ds(b0, nb), g, pl.ds(r0, nr)]
            else:
                src = (kb, vb)[a].at[pl.ds(b0, nb), 4 * g + slot, pl.ds(r0, nr)]
            dst = kv_buf.at[slot, a, pl.ds(b0, nb), pl.ds(r0, nr)]
            return pltpu.make_async_copy(src, dst, kv_sem(g, slot) if fin is None else fin_sem(fin))

        def w_copy(g, k, r0, nr):
            if k < 2:
                src = (wqa, wqb)[k].at[pl.ds(r0, nr), pl.ds(mo(g * 512, 512), 512)]
            else:
                src = (woa, wob)[k - 2].at[pl.ds(mo(g * 512 + r0, 8), nr)]
            return pltpu.make_async_copy(src, w_buf.at[g % 2, k, pl.ds(r0, nr)], w_sem(g))

        def x_copy(br, r0, nr):
            return pltpu.make_async_copy((xa, xb)[br].at[pl.ds(r0, nr)], x_buf.at[br, pl.ds(r0, nr)], w_sem(0))

        def start(mk, prio, *args):
            return lambda: mk(*args).start(priority=prio)

        def kv_main(g, slot, lo, hi):
            return [start(kv_copy, 1, g, slot, a, b0, 4, r0, 64) for r0 in range(lo, hi, 64) for a in (0, 1) for b0 in (0, 4)]

        def kv_fill(g, slot):
            return [start(kv_copy, 0, g, slot, a, b, 1, r0, hsm) for r0 in range(0, head, hsm) for b in range(NB) for a in (0, 1)]

        def w_fill(g, k):
            if k < 2:
                return [start(w_copy, 0, g, k, 64 * i + r0, 8) for r0 in range(0, 64, 8) for i in range(8)]
            return [start(w_copy, 0, g, k, r0, 8) for r0 in range(0, 512, 8)]

        def window(x_phase, y_phase, w):
            t1 = kv_main(*x_phase, ysplit, SK)
            if w is not None:
                return merge(t1 + kv_main(*y_phase, 0, ysplit), w_fill(*w), phase=(0.5, 0.75))
            return merge(t1 + kv_main(*y_phase, head, ysplit), kv_fill(*y_phase), phase=(0.5, 0.75))

        def fin_ops():
            ops = []
            x = kv_main(7, 2, ysplit, SK)
            if not xfill:
                ops, x = x, []
            for b0, arrs in ((0, (0, 1)), (4, (0,)), (4, (1,))):
                sem = lambda a, r0: 0 if b0 == 0 else (1 if a == 0 else (2 if r0 < vcut else 3))
                if fine and arrs == (1,):
                    t1 = [start(kv_copy, 1, 7, 3, 1, b0, 4, r0, 64, sem(1, r0)) for r0 in range(fhead, SK - fine, 64)]
                    t1 += [start(kv_copy, 1, 7, 3, 1, b, 1, r0, 64, sem(1, r0)) for r0 in range(SK - fine, SK, 64) for b in range(4, 8)]
                else:
                    t1 = [start(kv_copy, 1, 7, 3, a, b0, 4, r0, 64, sem(a, r0)) for r0 in range(fhead, SK, 64) for a in arrs]
                t0 = [start(kv_copy, 0, 7, 3, a, b, 1, r0, fhsm, sem(a, r0))
                      for r0 in range(0, fhead, fhsm) for b in range(b0, b0 + 4) for a in arrs]
                ops += merge(x + t1, t0, phase=(0.5, 0.25))
                x = []
            return ops

        def wait(ref, sem):
            if dma:
                pltpu.make_async_copy(ref, ref, sem).wait()

        def run_tasks(tasks, ops, npts=npoints):
            if not dma:
                ops = []
            if not compute or not ctx.get('c', True):
                for f in ops:
                    f()
                return
            total = sum(w for w, _ in tasks)
            pos, done, point = 0.0, 0, 0
            for w, fn in tasks:
                if point < npts and pos >= total * point / npts - 1e-9:
                    while point < npts and pos >= total * point / npts - 1e-9:
                        point += 1
                    upto = len(ops) * point // npts
                    for f in ops[done:upto]:
                        f()
                    done = upto
                fn()
                pos += w
            for f in ops[done:]:
                f()

        def a_tasks(g):
            st, T = {}, []
            par = g % 2

            def qproj(p):
                q = jnp.dot(x_buf[0, 96 * p:96 * (p + 1), :], w_buf[par, 0], preferred_element_type=f32)
                q = (q * QSCALE).astype(bf16)
                for u in range(2):
                    st["q", 2 * p + u] = jnp.concatenate(
                        [q[u * SQ:(u + 1) * SQ, i * DH:(i + 1) * DH] for i in range(4)], axis=0)

            def do_qk(b):
                st["s", b] = qk(st.pop(("q", b)), kv_buf[4, 0, b])

            def do_pv(b):
                st["o", b] = pv(*softmax_parts(st.pop(("s", b))), kv_buf[4, 1, b])

            def oproj(p):
                o = [st.pop(("o", 2 * p + u)) for u in range(2)]
                o = jnp.concatenate([jnp.concatenate([o[u][i * SQ:(i + 1) * SQ] for i in range(4)], axis=1)
                                     for u in range(2)], axis=0)
                acc_a[96 * p:96 * (p + 1), :] += jnp.dot(o, w_buf[par, 2], preferred_element_type=f32)

            T.append((384, lambda: qproj(0)))
            for b in range(NB + 1):
                if b < NB:
                    if b % 2 == 1 and b + 1 < NB:
                        T.append((384, lambda b=b: qproj((b + 1) // 2)))
                    T.append((400, lambda b=b: do_qk(b)))
                if b >= 1:
                    T.append((400, lambda b=b: do_pv(b - 1)))
                if b >= 3 and b % 2 == 1:
                    T.append((384, lambda b=b: oproj((b - 3) // 2)))
            T.append((384, lambda: oproj(3)))
            return T

        def b_qproj(g, j):
            q = jnp.dot(x_buf[1], w_buf[g % 2, 1, :, j * DH:(j + 1) * DH], preferred_element_type=f32)
            return (q * QSCALE).astype(bf16)

        def b_oproj(g, j, o, b0):
            rows = slice(b0 * SQ, (b0 + len(o)) * SQ)
            w = w_buf[g % 2, 3, j * DH:(j + 1) * DH, :]
            return jnp.dot(jnp.concatenate(o, axis=0), w, preferred_element_type=f32) + acc_b[rows, :]

        def b_tasks(g, j):
            st, T = {}, []

            def do_qk(b):
                st["s", b] = qk(st["q"][b * SQ:(b + 1) * SQ], kv_buf[j, 0, b])

            def do_pv(b):
                st["o", b] = pv(*softmax_parts(st.pop(("s", b))), kv_buf[j, 1, b])

            def oproj(b0):
                acc_b[b0 * SQ:(b0 + 4) * SQ, :] = b_oproj(g, j, [st.pop(("o", b)) for b in range(b0, b0 + 4)], b0)

            T.append((384, lambda: st.__setitem__("q", b_qproj(g, j))))
            for t in range(NB + skew):
                if t < NB:
                    T.append((128, lambda t=t: do_qk(t)))
                if t >= skew:
                    T.append((110, lambda t=t: do_pv(t - skew)))
                    if t - skew == 5:
                        T.append((192, lambda: oproj(0)))
            T.append((192, lambda: oproj(4)))
            return T

        def prologue():
            xs = [start(x_copy, 0, br, r0, 8) for r0 in range(0, M, 8) for br in (0, 1)]
            t1 = kv_main(0, 4, 0, SK)
            y = kv_main(0, 0, 0, ysplit)
            if pro_mode == 0:
                t0 = merge(xs, w_fill(0, 0), w_fill(0, 1), w_fill(0, 2), w_fill(0, 3))
                t1 = t1 + y
                ops = t1[:lead] + merge(t1[lead:], t0, phase=(0.5, 0.5))
            if dma:
                for f in ops:
                    f()
            acc_a[...] = jnp.zeros_like(acc_a)
            acc_b[...] = jnp.zeros_like(acc_b)
            wait(x_buf, w_sem(0))

        def a_phase(g, ops):
            wait(w_buf.at[g % 2], w_sem(g))
            wait(kv_buf.at[4], kv_sem(g, 4))
            ctx['c'] = bool(cmask & 1)
            run_tasks(a_tasks(g), ops, 2 * npoints)

        def b_phase(g, j, ops):
            wait(kv_buf.at[j], kv_sem(g, j))
            ctx['c'] = bool(cmask & 2)
            run_tasks(b_tasks(g, j), ops)

        def group(g):
            w1 = window((g, 1), (g, 2), (g + 1, 1))
            n = int(len(w1) * afrac)
            a_phase(g, window((g, 0), (g, 1), (g + 1, 0)) + w1[:n])
            b_phase(g, 0, w1[n:])
            b_phase(g, 1, window((g, 2), (g, 3), (g + 1, 2)))
            b_phase(g, 2, window((g, 3), (g + 1, 4), (g + 1, 3)))
            b_phase(g, 3, window((g + 1, 4), (g + 1, 0), None))

        def out_copy(r0, nr, c0, i):
            return pltpu.make_async_copy(out_buf.at[pl.ds(r0, nr), pl.ds(c0, D)], out.at[pl.ds(r0, nr), pl.ds(c0, D)], out_sem.at[i])

        def last_group():
            g = 7
            fin = fin_ops()
            ny = (SK - ysplit) // 16 + (len(fin) - (SK - ysplit) // 16) * ysplit // SK
            w1 = window((g, 1), (g, 2), None)
            n = int(len(w1) * afrac)
            a_phase(g, window((g, 0), (g, 1), None) + w1[:n])
            out_buf[:, 0:D] = acc_a[...].astype(bf16)
            b_phase(g, 0, w1[n:])
            b_phase(g, 1, fin[:ny])
            b_phase(g, 2, fin[ny:])
            compute = compute0 and bool(cmask & 4)
            qb = b_qproj(g, 3) if compute else None
            wait(kv_buf.at[3, :, pl.ds(0, 4)], fin_sem(0))
            for b0 in (0, 4):
                if b0 == 4:
                    wait(kv_buf.at[3, 0, pl.ds(4, 4)], fin_sem(1))
                if compute:
                    ps = [softmax_parts(s) for s in [qk(qb[b * SQ:(b + 1) * SQ], kv_buf[3, 0, b]) for b in range(b0, b0 + 4)]]
                if b0 == 4:
                    early = [out_copy(0, M, 0, 0), out_copy(0, 4 * SQ, D, 1)]
                    if wr_rows:
                        early = [pltpu.make_async_copy(out_buf.at[pl.ds(0, 4 * SQ)], out.at[pl.ds(0, 4 * SQ)], out_sem.at[0]),
                                 out_copy(4 * SQ, 4 * SQ, 0, 1)]
                    wait(kv_buf.at[3, 1, pl.ds(4, 4), pl.ds(0, vcut)], fin_sem(2))
                    for c in early:
                        c.start()
                    if compute and pvsplit:
                        part = [jnp.dot(ps[i][0][:, :vcut], kv_buf[3, 1, b0 + i, :vcut, :], preferred_element_type=f32) for i in range(4)]
                    wait(kv_buf.at[3, 1, pl.ds(4, 4), pl.ds(vcut, SK - vcut)], fin_sem(3))
                rows = slice(b0 * SQ, (b0 + 4) * SQ)
                if compute and pvsplit and b0 == 4:
                    o = [part[i] + jnp.dot(ps[i][0][:, vcut:], kv_buf[3, 1, b0 + i, vcut:, :], preferred_element_type=f32) for i in range(4)]
                    r = b_oproj(g, 3, [(o[i] * (1.0 / ps[i][1])).astype(bf16) for i in range(4)], b0)
                elif compute:
                    r = b_oproj(g, 3, [pv(*ps[i], kv_buf[3, 1, b0 + i]) for i in range(4)], b0)
                else:
                    r = acc_b[rows, :]
                out_buf[rows, D:2 * D] = r.astype(bf16)
            oc = out_copy(4 * SQ, 4 * SQ, D, 2)
            oc.start()
            for c in early + [oc]:
                c.wait()

        def body(i, c):
            @pl.when(i == 0)
            def _():
                ctx["z"] = i
                prologue()

            @pl.when(i < G - 1)
            def _():
                ctx["z"] = 0
                group(i)

            @pl.when(i == G - 1)
            def _():
                ctx["z"] = i - (G - 1)
                last_group()
            return c

        jax.lax.fori_loop(0, G, body, 0)

    def fn(A_x, A_k, A_v, A_wq, A_wo, B_x, B_k, B_v, B_wq, B_wo):
        out = pl.pallas_call(
            kernel,
            in_specs=[pl.BlockSpec(memory_space=pltpu.HBM)] * 10,
            out_specs=pl.BlockSpec(memory_space=pltpu.HBM),
            out_shape=jax.ShapeDtypeStruct((M, 2 * D), bf16),
            scratch_shapes=[
                pltpu.VMEM((5, 2, NB, SK, DH), bf16),
                pltpu.VMEM((2, M, D), bf16),
                pltpu.VMEM((2, 4, 512, 512), bf16),
                pltpu.VMEM((M, D), f32),
                pltpu.VMEM((M, D), f32),
                pltpu.VMEM((M, 2 * D), bf16),
                pltpu.SemaphoreType.DMA((10 + G + 4,)),
                pltpu.SemaphoreType.DMA((3,)),
            ],
            compiler_params=pltpu.CompilerParams(vmem_limit_bytes=64 * 2**20, disable_bounds_checks=nobounds,
                                                 disable_semaphore_checks=nosem),
            name=name,
        )(A_x.reshape(M, D), A_k, A_v, A_wq, A_wo, B_x.reshape(M, D), B_k, B_v, B_wq, B_wo)
        return out.reshape(NB, SQ, 2 * D)
    return fn


@jax.jit
def pallas_concat_heads__gqa_block_cached__mha_block_cached__near_ridge_kernel(
    A_x, A_k_cache, A_v_cache, A_wq, A_wo, B_x, B_k_cache, B_v_cache, B_wq, B_wo):
    return build()(A_x, A_k_cache, A_v_cache, A_wq, A_wo, B_x, B_k_cache, B_v_cache, B_wq, B_wo)
```

```python
import math

import jax
import jax.numpy as jnp
import jax.experimental.pallas as pl
import jax.experimental.pallas.tpu as pltpu

BATCH, SQ, D = 8, 48, 512
SK, DH = 1024, 128
GROUPS = 8
GROUP_W = 4 * DH
M = BATCH * SQ
Q_SCALE = DH ** -0.5 * math.log2(math.e)

GQA_SLOT = 4
BULK, FILL = 1, 0
AHEAD_ROWS = 832
QUEUE_DEPTH = 27
LAST_FILL_ROWS = 128
LAST_V_CUT = 768

SEM_KV, SEM_W, SEM_X, SEM_LAST, NUM_SEMS = 0, 10, 18, 19, 23

f32, bf16 = jnp.float32, jnp.bfloat16


def _dot(a, b):
    return jnp.dot(a, b, preferred_element_type=f32)


def _scores(q, k):
    return jax.lax.dot_general(q, k, (((1,), (1,)), ((), ())), preferred_element_type=f32)


def _exp_and_sum(s):
    p = jnp.exp2(s - jnp.max(s, axis=-1, keepdims=True))
    return p.astype(bf16), jnp.sum(p, axis=-1, keepdims=True)


def _normalize(o, denom):
    return (o * (1.0 / denom)).astype(bf16)


def _interleave(*seqs):
    keyed = [((i + 0.5) / len(seq), w, i) for w, seq in enumerate(seqs) for i in range(len(seq))]
    return [seqs[w][i] for _, w, i in sorted(keyed)]


def _run(stages, starts, points):
    total = sum(cost for cost, _ in stages)
    spent, started, point = 0, 0, 0
    for cost, stage in stages:
        while point < points and spent * points >= total * point:
            point += 1
        upto = len(starts) * point // points
        for start in starts[started:upto]:
            start()
        started = upto
        stage()
        spent += cost
    for start in starts[started:]:
        start()


def _kernel(xa_hbm, ka_hbm, va_hbm, wqa_hbm, woa_hbm, xb_hbm, kb_hbm, vb_hbm, wqb_hbm, wob_hbm, out_hbm,
            kv_buf, x_buf, w_buf, acc_a, acc_b, ya_buf, yb0_buf, yb1_buf, sems, out_sems):

    class Copies:
        def __init__(self, zero):
            self.zero = zero

        def sem(self, i):
            return sems.at[i + self.zero]

        def kv_sem(self, g, slot):
            return self.sem(SEM_KV + 5 * (g % 2) + slot)

        def kv(self, priority, g, slot, kv, b0, nb, r0, nr, sem=None):
            def start():
                if slot == GQA_SLOT:
                    src = (ka_hbm, va_hbm)[kv].at[pl.ds(b0, nb), g, pl.ds(r0, nr)]
                else:
                    src = (kb_hbm, vb_hbm)[kv].at[pl.ds(b0, nb), 4 * g + slot, pl.ds(r0, nr)]
                dst = kv_buf.at[slot, kv, pl.ds(b0, nb), pl.ds(r0, nr)]
                s = self.kv_sem(g, slot) if sem is None else self.sem(sem)
                pltpu.make_async_copy(src, dst, s).start(priority=priority)
            return start

        def bulk(self, g, slot, batches, lo, hi):
            return [self.kv(BULK, g, slot, kv, b0, min(4, batches - b0), r0, 64)
                    for r0 in range(lo, hi, 64) for kv in (0, 1) for b0 in (0, 4)]

        def last_batch(self, g, slot):
            return [self.kv(FILL, g, slot, kv, BATCH - 1, 1, r0 + r, 32)
                    for r0 in range(0, SK, 64) for kv in (0, 1) for r in (0, 32)]

        def weights(self, g, which, priority=FILL, nr=8):
            def piece(r0):
                def start():
                    base = g * GROUP_W if isinstance(g, int) else pl.multiple_of(g * GROUP_W, GROUP_W)
                    if which < 2:
                        src = (wqa_hbm, wqb_hbm)[which].at[pl.ds(r0, nr), pl.ds(base, GROUP_W)]
                    else:
                        src = (woa_hbm, wob_hbm)[which - 2].at[pl.ds(base + r0, nr)]
                    dst = w_buf.at[g % 2, which, pl.ds(r0, nr)]
                    pltpu.make_async_copy(src, dst, self.sem(SEM_W + g)).start(priority=priority)
                return start
            if which < 2:
                return [piece(64 * i + r0) for r0 in range(0, 64, nr) for i in range(8)]
            return [piece(r0) for r0 in range(0, GROUP_W, nr)]

        def x(self):
            def piece(br, r0):
                def start():
                    src = (xa_hbm, xb_hbm)[br].at[pl.ds(r0, 16)]
                    pltpu.make_async_copy(src, x_buf.at[br, pl.ds(r0, 16)], self.sem(SEM_X)).start(priority=BULK)
                return start
            return [piece(br, r0) for r0 in range(0, M, 16) for br in (0, 1)]

        def window(self, nxt, after, weights=None):
            fill = self.last_batch(*after[:2]) if weights is None else self.weights(*weights)
            bulk = self.bulk(*nxt, AHEAD_ROWS, SK) + self.bulk(*after, 0, AHEAD_ROWS)
            return _interleave(bulk, fill)

        def last_head(self):
            g, fill = GROUPS - 1, []
            bulk = self.bulk(g, 2, BATCH - 1, AHEAD_ROWS, SK)
            for b0, kvs in ((0, (0, 1)), (4, (0,)), (4, (1,))):
                def sem(kv, r0):
                    return SEM_LAST + (0 if b0 == 0 else 1 if kv == 0 else 2 if r0 < LAST_V_CUT else 3)
                bulk += [self.kv(BULK, g, 3, kv, b0, 4, r0, 64, sem(kv, r0))
                         for r0 in range(LAST_FILL_ROWS, SK, 64) for kv in kvs]
                fill += [self.kv(FILL, g, 3, kv, b, 1, r0, 32, sem(kv, r0))
                         for r0 in range(0, LAST_FILL_ROWS, 32) for b in range(b0, b0 + 4) for kv in kvs]
            return _interleave(bulk, fill)

    def wait_filled(ref, sem):
        pltpu.make_async_copy(ref, ref, sem).wait()

    def gqa_phase(copies, g, starts):
        live = {}

        def q_proj(pair):
            q = (_dot(x_buf[0, 2 * SQ * pair:2 * SQ * (pair + 1), :], w_buf[g % 2, 0]) * Q_SCALE).astype(bf16)
            for u in range(2):
                live["q", 2 * pair + u] = jnp.concatenate(
                    [q[u * SQ:(u + 1) * SQ, i * DH:(i + 1) * DH] for i in range(4)], axis=0)

        def qk(b):
            live["s", b] = _scores(live.pop(("q", b)), kv_buf[GQA_SLOT, 0, b])

        def pv(b):
            p, denom = _exp_and_sum(live.pop(("s", b)))
            live["o", b] = _normalize(_dot(p, kv_buf[GQA_SLOT, 1, b]), denom)

        def o_proj(pair):
            o = [live.pop(("o", 2 * pair + u)) for u in range(2)]
            o = jnp.concatenate(
                [jnp.concatenate([ou[i * SQ:(i + 1) * SQ] for i in range(4)], axis=1) for ou in o], axis=0)
            acc_a[2 * SQ * pair:2 * SQ * (pair + 1), :] += _dot(o, w_buf[g % 2, 2])

        stages = [(384, lambda: q_proj(0))]
        for b in range(BATCH + 1):
            if b % 2 == 1 and b + 1 < BATCH:
                stages.append((384, lambda b=b: q_proj((b + 1) // 2)))
            if b < BATCH:
                stages.append((400, lambda b=b: qk(b)))
            if b >= 1:
                stages.append((400, lambda b=b: pv(b - 1)))
            if b % 2 == 1 and b >= 3:
                stages.append((384, lambda b=b: o_proj((b - 3) // 2)))
        stages.append((384, lambda: o_proj(3)))

        wait_filled(w_buf.at[g % 2], copies.sem(SEM_W + g))
        wait_filled(kv_buf.at[GQA_SLOT], copies.kv_sem(g, GQA_SLOT))
        _run(stages, starts, 8)

    def mha_q(g, j):
        return (_dot(x_buf[1], w_buf[g % 2, 1, :, j * DH:(j + 1) * DH]) * Q_SCALE).astype(bf16)

    def mha_y(g, j, b0, o):
        w = w_buf[g % 2, 3, j * DH:(j + 1) * DH, :]
        return _dot(jnp.concatenate(o, axis=0), w) + acc_b[b0 * SQ:(b0 + 4) * SQ, :]

    def mha_phase(copies, g, j, starts):
        live = {}

        def q_proj():
            live["q"] = mha_q(g, j)

        def qk(b):
            live["s", b] = _scores(live["q"][b * SQ:(b + 1) * SQ], kv_buf[j, 0, b])

        def pv(b):
            p, denom = _exp_and_sum(live.pop(("s", b)))
            live["o", b] = _normalize(_dot(p, kv_buf[j, 1, b]), denom)

        def o_proj(b0):
            acc_b[b0 * SQ:(b0 + 4) * SQ, :] = mha_y(g, j, b0, [live.pop(("o", b)) for b in range(b0, b0 + 4)])

        stages = [(384, q_proj)]
        for b in range(BATCH + 2):
            if b < BATCH:
                stages.append((128, lambda b=b: qk(b)))
            if b >= 2:
                stages.append((110, lambda b=b: pv(b - 2)))
            if b == BATCH - 1:
                stages.append((192, lambda: o_proj(0)))
        stages.append((192, lambda: o_proj(4)))

        wait_filled(kv_buf.at[j], copies.kv_sem(g, j))
        _run(stages, starts, 4)

    def prologue(copies):
        first = copies.bulk(0, GQA_SLOT, BATCH, 0, SK)
        small = _interleave(copies.x(), copies.weights(0, 2, BULK, 16), copies.weights(0, 3, BULK, 16))
        fill = copies.weights(0, 0) + copies.weights(0, 1)
        paired = len(first) - QUEUE_DEPTH
        starts = (first[:QUEUE_DEPTH] + _interleave(first[QUEUE_DEPTH:], fill[:paired])
                  + _interleave(small, fill[paired:])
                  + _interleave(copies.bulk(0, 0, BATCH - 1, 0, AHEAD_ROWS), copies.last_batch(0, 0)))
        for start in starts:
            start()
        acc_a[...] = jnp.zeros_like(acc_a)
        acc_b[...] = jnp.zeros_like(acc_b)
        wait_filled(x_buf, copies.sem(SEM_X))

    def first_two_phases(copies, g, window_a, window_0):
        early = len(window_0) // 4
        gqa_phase(copies, g, window_a + window_0[:early])
        mha_phase(copies, g, 0, window_0[early:])

    def group(copies, g):
        phases = [(g, 0, BATCH - 1), (g, 1, BATCH), (g, 2, BATCH), (g, 3, BATCH),
                  (g + 1, GQA_SLOT, BATCH), (g + 1, 0, BATCH - 1)]
        windows = [copies.window(phases[i], phases[i + 1], (g + 1, i) if i < 4 else None) for i in range(5)]
        first_two_phases(copies, g, windows[0], windows[1])
        for j in range(1, 4):
            mha_phase(copies, g, j, windows[j + 1])

    def last_group(copies):
        g = GROUPS - 1
        phases = [(g, j, BATCH - 1) for j in range(3)]
        first_two_phases(copies, g, copies.window(phases[0], phases[1]), copies.window(phases[1], phases[2]))
        ya_buf[...] = acc_a[...].astype(bf16)
        starts = copies.last_head()
        cut = len(starts) * AHEAD_ROWS // SK
        mha_phase(copies, g, 1, starts[:cut])
        mha_phase(copies, g, 2, starts[cut:])

        q = mha_q(g, 3)

        def probs(b0):
            s = [_scores(q[b * SQ:(b + 1) * SQ], kv_buf[3, 0, b]) for b in range(b0, b0 + 4)]
            return [_exp_and_sum(sb) for sb in s]

        def finish(b0, p, y_buf):
            o = [_normalize(_dot(pb, kv_buf[3, 1, b0 + i]), denom) for i, (pb, denom) in enumerate(p)]
            y_buf[...] = mha_y(g, 3, b0, o).astype(bf16)

        half = 4 * SQ
        writes = [
            pltpu.make_async_copy(ya_buf, out_hbm.at[:, pl.ds(0, D)], out_sems.at[0]),
            pltpu.make_async_copy(yb0_buf, out_hbm.at[pl.ds(0, half), pl.ds(D, D)], out_sems.at[1]),
            pltpu.make_async_copy(yb1_buf, out_hbm.at[pl.ds(half, half), pl.ds(D, D)], out_sems.at[2]),
        ]
        wait_filled(kv_buf.at[3, :, pl.ds(0, 4)], copies.sem(SEM_LAST))
        finish(0, probs(0), yb0_buf)
        wait_filled(kv_buf.at[3, 0, pl.ds(4, 4)], copies.sem(SEM_LAST + 1))
        p = probs(4)
        wait_filled(kv_buf.at[3, 1, pl.ds(4, 4), pl.ds(0, LAST_V_CUT)], copies.sem(SEM_LAST + 2))
        writes[0].start()
        writes[1].start()
        wait_filled(kv_buf.at[3, 1, pl.ds(4, 4), pl.ds(LAST_V_CUT, SK - LAST_V_CUT)], copies.sem(SEM_LAST + 3))
        finish(4, p, yb1_buf)
        writes[2].start()
        for write in writes:
            write.wait()

    def body(g, carry):
        @pl.when(g == 0)
        def _():
            prologue(Copies(g))

        @pl.when(g < GROUPS - 1)
        def _():
            group(Copies(0), g)

        @pl.when(g == GROUPS - 1)
        def _():
            last_group(Copies(g - (GROUPS - 1)))

        return carry

    jax.lax.fori_loop(0, GROUPS, body, 0)


@jax.jit
def pallas_concat_heads__gqa_block_cached__mha_block_cached__near_ridge_kernel(
    A_x: jax.Array,
    A_k_cache: jax.Array,
    A_v_cache: jax.Array,
    A_wq: jax.Array,
    A_wo: jax.Array,
    B_x: jax.Array,
    B_k_cache: jax.Array,
    B_v_cache: jax.Array,
    B_wq: jax.Array,
    B_wo: jax.Array,
):
    out = pl.pallas_call(
        _kernel,
        in_specs=[pl.BlockSpec(memory_space=pltpu.HBM)] * 10,
        out_specs=pl.BlockSpec(memory_space=pltpu.HBM),
        out_shape=jax.ShapeDtypeStruct((M, 2 * D), bf16),
        scratch_shapes=[
            pltpu.VMEM((5, 2, BATCH, SK, DH), bf16),
            pltpu.VMEM((2, M, D), bf16),
            pltpu.VMEM((2, 4, GROUP_W, D), bf16),
            pltpu.VMEM((M, D), f32),
            pltpu.VMEM((M, D), f32),
            pltpu.VMEM((M, D), bf16),
            pltpu.VMEM((M // 2, D), bf16),
            pltpu.VMEM((M // 2, D), bf16),
            pltpu.SemaphoreType.DMA((NUM_SEMS,)),
            pltpu.SemaphoreType.DMA((3,)),
        ],
        compiler_params=pltpu.CompilerParams(
            vmem_limit_bytes=64 * 2 ** 20,
            disable_bounds_checks=True,
            disable_semaphore_checks=True,
        ),
        name="gqa_mha_cached_blocks",
    )(A_x.reshape(M, D), A_k_cache, A_v_cache, A_wq, A_wo,
      B_x.reshape(M, D), B_k_cache, B_v_cache, B_wq, B_wo)
    return out.reshape(BATCH, SQ, 2 * D)
```

```python
import math

import jax
import jax.numpy as jnp
import jax.experimental.pallas as pl
import jax.experimental.pallas.tpu as pltpu

BATCH, SQ, D = 8, 48, 512
SK, DH = 1024, 128
GROUPS = 8
GROUP_W = 4 * DH
M = BATCH * SQ
Q_SCALE = DH ** -0.5 * math.log2(math.e)

GQA_SLOT = 4
BULK, FILL = 1, 0
AHEAD_ROWS = 768
LEAD = 16
LAST_FILL_ROWS = 128
LAST_V_CUT = 768

SEM_KV, SEM_W, SEM_X, SEM_LAST, NUM_SEMS = 0, 10, 18, 19, 23

f32, bf16 = jnp.float32, jnp.bfloat16


def _dot(a, b):
    return jnp.dot(a, b, preferred_element_type=f32)


def _scores(q, k):
    return jax.lax.dot_general(q, k, (((1,), (1,)), ((), ())), preferred_element_type=f32)


def _exp_and_sum(s):
    p = jnp.exp2(s - jnp.max(s, axis=-1, keepdims=True))
    return p.astype(bf16), jnp.sum(p, axis=-1, keepdims=True)


def _normalize(o, denom):
    return (o * (1.0 / denom)).astype(bf16)


def _interleave(*seqs):
    keyed = [((i + 0.5) / len(seq), w, i) for w, seq in enumerate(seqs) for i in range(len(seq))]
    return [seqs[w][i] for _, w, i in sorted(keyed)]


def _run(stages, starts, points):
    total = sum(cost for cost, _ in stages)
    spent, started, point = 0, 0, 0
    for cost, stage in stages:
        while point < points and spent * points >= total * point:
            point += 1
        upto = len(starts) * point // points
        for start in starts[started:upto]:
            start()
        started = upto
        stage()
        spent += cost
    for start in starts[started:]:
        start()


def _kernel(xa_hbm, ka_hbm, va_hbm, wqa_hbm, woa_hbm, xb_hbm, kb_hbm, vb_hbm, wqb_hbm, wob_hbm, out_hbm,
            kv_buf, x_buf, w_buf, acc_a, acc_b, ya_buf, yb0_buf, yb1_buf, sems, out_sems):

    class Copies:
        def __init__(self, zero):
            self.zero = zero

        def sem(self, i):
            return sems.at[i + self.zero]

        def kv_sem(self, g, slot):
            return self.sem(SEM_KV + 5 * (g % 2) + slot)

        def kv(self, priority, g, slot, kv, b0, nb, r0, nr, sem=None):
            def start():
                if slot == GQA_SLOT:
                    src = (ka_hbm, va_hbm)[kv].at[pl.ds(b0, nb), g, pl.ds(r0, nr)]
                else:
                    src = (kb_hbm, vb_hbm)[kv].at[pl.ds(b0, nb), 4 * g + slot, pl.ds(r0, nr)]
                dst = kv_buf.at[slot, kv, pl.ds(b0, nb), pl.ds(r0, nr)]
                s = self.kv_sem(g, slot) if sem is None else self.sem(sem)
                pltpu.make_async_copy(src, dst, s).start(priority=priority)
            return start

        def bulk(self, g, slot, first, lo, hi):
            return [self.kv(BULK, g, slot, kv, b0, min(4, BATCH - b0), r0, 64)
                    for r0 in range(lo, hi, 64) for kv in (0, 1) for b0 in (first, first + 4)]

        def batch0(self, g, slot):
            return [self.kv(FILL, g, slot, kv, 0, 1, r0 + r, 32)
                    for r0 in range(0, SK, 64) for kv in (0, 1) for r in (0, 32)]

        def weights(self, g, which, priority=FILL, nr=8):
            def piece(r0):
                def start():
                    base = g * GROUP_W if isinstance(g, int) else pl.multiple_of(g * GROUP_W, GROUP_W)
                    if which < 2:
                        src = (wqa_hbm, wqb_hbm)[which].at[pl.ds(r0, nr), pl.ds(base, GROUP_W)]
                    else:
                        src = (woa_hbm, wob_hbm)[which - 2].at[pl.ds(base + r0, nr)]
                    dst = w_buf.at[g % 2, which, pl.ds(r0, nr)]
                    pltpu.make_async_copy(src, dst, self.sem(SEM_W + g)).start(priority=priority)
                return start
            if which < 2:
                return [piece(64 * i + r0) for r0 in range(0, 64, nr) for i in range(8)]
            return [piece(r0) for r0 in range(0, GROUP_W, nr)]

        def x(self):
            def piece(br, r0):
                def start():
                    src = (xa_hbm, xb_hbm)[br].at[pl.ds(r0, 16)]
                    pltpu.make_async_copy(src, x_buf.at[br, pl.ds(r0, 16)], self.sem(SEM_X)).start(priority=BULK)
                return start
            return [piece(br, r0) for r0 in range(0, M, 16) for br in (0, 1)]

        def window(self, nxt, after, weights=None):
            fill = self.batch0(*after[:2]) if weights is None else self.weights(*weights)
            bulk = self.bulk(*nxt, AHEAD_ROWS, SK) + self.bulk(*after, 0, AHEAD_ROWS)
            return _interleave(bulk, fill)

        def last_head(self):
            g, fill = GROUPS - 1, []
            bulk = self.bulk(g, 2, 1, AHEAD_ROWS, SK)
            for b0, kvs in ((0, (0, 1)), (4, (0,)), (4, (1,))):
                def sem(kv, r0):
                    return SEM_LAST + (0 if b0 == 0 else 1 if kv == 0 else 2 if r0 < LAST_V_CUT else 3)
                bulk += [self.kv(BULK, g, 3, kv, b0, 4, r0, 64, sem(kv, r0))
                         for r0 in range(LAST_FILL_ROWS, SK, 64) for kv in kvs]
                fill += [self.kv(FILL, g, 3, kv, b, 1, r0, 32, sem(kv, r0))
                         for r0 in range(0, LAST_FILL_ROWS, 32) for b in range(b0, b0 + 4) for kv in kvs]
            return _interleave(bulk, fill)

    def wait_filled(ref, sem):
        pltpu.make_async_copy(ref, ref, sem).wait()

    def gqa_phase(copies, g, starts):
        live = {}

        def q_proj(pair):
            q = (_dot(x_buf[0, 2 * SQ * pair:2 * SQ * (pair + 1), :], w_buf[g % 2, 0]) * Q_SCALE).astype(bf16)
            for u in range(2):
                live["q", 2 * pair + u] = jnp.concatenate(
                    [q[u * SQ:(u + 1) * SQ, i * DH:(i + 1) * DH] for i in range(4)], axis=0)

        def qk(b):
            live["s", b] = _scores(live.pop(("q", b)), kv_buf[GQA_SLOT, 0, b])

        def pv(b):
            p, denom = _exp_and_sum(live.pop(("s", b)))
            live["o", b] = _normalize(_dot(p, kv_buf[GQA_SLOT, 1, b]), denom)

        def o_proj(pair):
            o = [live.pop(("o", 2 * pair + u)) for u in range(2)]
            o = jnp.concatenate(
                [jnp.concatenate([ou[i * SQ:(i + 1) * SQ] for i in range(4)], axis=1) for ou in o], axis=0)
            acc_a[2 * SQ * pair:2 * SQ * (pair + 1), :] += _dot(o, w_buf[g % 2, 2])

        stages = [(384, lambda: q_proj(0))]
        for b in range(BATCH + 1):
            if b % 2 == 1 and b + 1 < BATCH:
                stages.append((384, lambda b=b: q_proj((b + 1) // 2)))
            if b < BATCH:
                stages.append((400, lambda b=b: qk(b)))
            if b >= 1:
                stages.append((400, lambda b=b: pv(b - 1)))
            if b % 2 == 1 and b >= 3:
                stages.append((384, lambda b=b: o_proj((b - 3) // 2)))
        stages.append((384, lambda: o_proj(3)))

        wait_filled(w_buf.at[g % 2], copies.sem(SEM_W + g))
        wait_filled(kv_buf.at[GQA_SLOT], copies.kv_sem(g, GQA_SLOT))
        _run(stages, starts, 8)

    def mha_q(g, j):
        return (_dot(x_buf[1], w_buf[g % 2, 1, :, j * DH:(j + 1) * DH]) * Q_SCALE).astype(bf16)

    def mha_y(g, j, b0, o):
        w = w_buf[g % 2, 3, j * DH:(j + 1) * DH, :]
        return _dot(jnp.concatenate(o, axis=0), w) + acc_b[b0 * SQ:(b0 + 4) * SQ, :]

    def mha_phase(copies, g, j, starts):
        live = {}

        def q_proj():
            live["q"] = mha_q(g, j)

        def qk(b):
            live["s", b] = _scores(live["q"][b * SQ:(b + 1) * SQ], kv_buf[j, 0, b])

        def pv(b):
            p, denom = _exp_and_sum(live.pop(("s", b)))
            live["o", b] = _normalize(_dot(p, kv_buf[j, 1, b]), denom)

        def o_proj(b0):
            acc_b[b0 * SQ:(b0 + 4) * SQ, :] = mha_y(g, j, b0, [live.pop(("o", b)) for b in range(b0, b0 + 4)])

        stages = [(384, q_proj)]
        for b in range(BATCH + 2):
            if b < BATCH:
                stages.append((128, lambda b=b: qk(b)))
            if b >= 2:
                stages.append((110, lambda b=b: pv(b - 2)))
            if b == BATCH - 1:
                stages.append((192, lambda: o_proj(0)))
        stages.append((192, lambda: o_proj(4)))

        wait_filled(kv_buf.at[j], copies.kv_sem(g, j))
        _run(stages, starts, 4)

    def prologue(copies):
        first = copies.bulk(0, GQA_SLOT, 0, 0, SK)
        small = _interleave(copies.x(), copies.weights(0, 2, BULK, 16), copies.weights(0, 3, BULK, 16))
        fill = copies.weights(0, 0) + copies.weights(0, 1)
        paired = len(first) - LEAD
        starts = (first[:LEAD] + _interleave(first[LEAD:], fill[:paired])
                  + _interleave(small, fill[paired:])
                  + _interleave(copies.bulk(0, 0, 1, 0, AHEAD_ROWS), copies.batch0(0, 0)))
        for start in starts:
            start()
        acc_a[...] = jnp.zeros_like(acc_a)
        acc_b[...] = jnp.zeros_like(acc_b)
        wait_filled(x_buf, copies.sem(SEM_X))

    def first_two_phases(copies, g, window_a, window_0):
        early = len(window_0) // 4
        gqa_phase(copies, g, window_a + window_0[:early])
        mha_phase(copies, g, 0, window_0[early:])

    def group(copies, g):
        phases = [(g, 0, 1), (g, 1, 0), (g, 2, 0), (g, 3, 0), (g + 1, GQA_SLOT, 0), (g + 1, 0, 1)]
        windows = [copies.window(phases[i], phases[i + 1], (g + 1, i) if i < 4 else None) for i in range(5)]
        first_two_phases(copies, g, windows[0], windows[1])
        for j in range(1, 4):
            mha_phase(copies, g, j, windows[j + 1])

    def last_group(copies):
        g = GROUPS - 1
        phases = [(g, j, 1) for j in range(3)]
        first_two_phases(copies, g, copies.window(phases[0], phases[1]), copies.window(phases[1], phases[2]))
        ya_buf[...] = acc_a[...].astype(bf16)
        starts = copies.last_head()
        cut = len(starts) * AHEAD_ROWS // SK
        mha_phase(copies, g, 1, starts[:cut])
        mha_phase(copies, g, 2, starts[cut:])

        q = mha_q(g, 3)

        def probs(b0):
            s = [_scores(q[b * SQ:(b + 1) * SQ], kv_buf[3, 0, b]) for b in range(b0, b0 + 4)]
            return [_exp_and_sum(sb) for sb in s]

        def finish(b0, p, y_buf):
            o = [_normalize(_dot(pb, kv_buf[3, 1, b0 + i]), denom) for i, (pb, denom) in enumerate(p)]
            y_buf[...] = mha_y(g, 3, b0, o).astype(bf16)

        half = 4 * SQ
        writes = [
            pltpu.make_async_copy(ya_buf, out_hbm.at[:, pl.ds(0, D)], out_sems.at[0]),
            pltpu.make_async_copy(yb0_buf, out_hbm.at[pl.ds(0, half), pl.ds(D, D)], out_sems.at[1]),
            pltpu.make_async_copy(yb1_buf, out_hbm.at[pl.ds(half, half), pl.ds(D, D)], out_sems.at[2]),
        ]
        wait_filled(kv_buf.at[3, :, pl.ds(0, 4)], copies.sem(SEM_LAST))
        finish(0, probs(0), yb0_buf)
        wait_filled(kv_buf.at[3, 0, pl.ds(4, 4)], copies.sem(SEM_LAST + 1))
        p = probs(4)
        wait_filled(kv_buf.at[3, 1, pl.ds(4, 4), pl.ds(0, LAST_V_CUT)], copies.sem(SEM_LAST + 2))
        writes[0].start()
        writes[1].start()
        wait_filled(kv_buf.at[3, 1, pl.ds(4, 4), pl.ds(LAST_V_CUT, SK - LAST_V_CUT)], copies.sem(SEM_LAST + 3))
        finish(4, p, yb1_buf)
        writes[2].start()
        for write in writes:
            write.wait()

    def body(g, carry):
        @pl.when(g == 0)
        def _():
            prologue(Copies(g))

        @pl.when(g < GROUPS - 1)
        def _():
            group(Copies(0), g)

        @pl.when(g == GROUPS - 1)
        def _():
            last_group(Copies(g - (GROUPS - 1)))

        return carry

    jax.lax.fori_loop(0, GROUPS, body, 0)


@jax.jit
def pallas_concat_heads__gqa_block_cached__mha_block_cached__near_ridge_kernel(
    A_x: jax.Array,
    A_k_cache: jax.Array,
    A_v_cache: jax.Array,
    A_wq: jax.Array,
    A_wo: jax.Array,
    B_x: jax.Array,
    B_k_cache: jax.Array,
    B_v_cache: jax.Array,
    B_wq: jax.Array,
    B_wo: jax.Array,
):
    out = pl.pallas_call(
        _kernel,
        in_specs=[pl.BlockSpec(memory_space=pltpu.HBM)] * 10,
        out_specs=pl.BlockSpec(memory_space=pltpu.HBM),
        out_shape=jax.ShapeDtypeStruct((M, 2 * D), bf16),
        scratch_shapes=[
            pltpu.VMEM((5, 2, BATCH, SK, DH), bf16),
            pltpu.VMEM((2, M, D), bf16),
            pltpu.VMEM((2, 4, GROUP_W, D), bf16),
            pltpu.VMEM((M, D), f32),
            pltpu.VMEM((M, D), f32),
            pltpu.VMEM((M, D), bf16),
            pltpu.VMEM((M // 2, D), bf16),
            pltpu.VMEM((M // 2, D), bf16),
            pltpu.SemaphoreType.DMA((NUM_SEMS,)),
            pltpu.SemaphoreType.DMA((3,)),
        ],
        compiler_params=pltpu.CompilerParams(
            vmem_limit_bytes=64 * 2 ** 20,
            disable_bounds_checks=True,
            disable_semaphore_checks=True,
        ),
        name="gqa_mha_cached_blocks",
    )(A_x.reshape(M, D), A_k_cache, A_v_cache, A_wq, A_wo,
      B_x.reshape(M, D), B_k_cache, B_v_cache, B_wq, B_wo)
    return out.reshape(BATCH, SQ, 2 * D)
```

```python
import math

import jax
import jax.numpy as jnp
import jax.experimental.pallas as pl
import jax.experimental.pallas.tpu as pltpu

BATCH, SQ, D = 8, 48, 512
SK, DH = 1024, 128
GROUPS = 8
GROUP_W = 4 * DH
M = BATCH * SQ
Q_SCALE = DH ** -0.5 * math.log2(math.e)

GQA_SLOT = 4
BULK, FILL = 1, 0
AHEAD_ROWS = 768
LEAD = 16
LAST_FILL_ROWS = 128
LAST_PARTS = ((0, 4), (4, 2), (6, 2))
LAST_V_CUT = 384

SEM_KV, SEM_W, SEM_X, SEM_LAST, NUM_SEMS = 0, 10, 18, 19, 24

f32, bf16 = jnp.float32, jnp.bfloat16


def _dot(a, b):
    return jnp.dot(a, b, preferred_element_type=f32)


def _scores(q, k):
    return jax.lax.dot_general(q, k, (((1,), (1,)), ((), ())), preferred_element_type=f32)


def _exp_and_sum(s):
    p = jnp.exp2(s - jnp.max(s, axis=-1, keepdims=True))
    return p.astype(bf16), jnp.sum(p, axis=-1, keepdims=True)


def _normalize(o, denom):
    return (o * (1.0 / denom)).astype(bf16)


def _interleave(*seqs):
    keyed = [((i + 0.5) / len(seq), w, i) for w, seq in enumerate(seqs) for i in range(len(seq))]
    return [seqs[w][i] for _, w, i in sorted(keyed)]


def _run(stages, starts, points):
    total = sum(cost for cost, _ in stages)
    spent, started, point = 0, 0, 0
    for cost, stage in stages:
        while point < points and spent * points >= total * point:
            point += 1
        upto = len(starts) * point // points
        for start in starts[started:upto]:
            start()
        started = upto
        stage()
        spent += cost
    for start in starts[started:]:
        start()


def _kernel(xa_hbm, ka_hbm, va_hbm, wqa_hbm, woa_hbm, xb_hbm, kb_hbm, vb_hbm, wqb_hbm, wob_hbm, out_hbm,
            kv_buf, x_buf, w_buf, acc_a, acc_b, sems, out_sems, ya_buf, *yb_bufs):

    class Copies:
        def __init__(self, zero):
            self.zero = zero

        def sem(self, i):
            return sems.at[i + self.zero]

        def kv_sem(self, g, slot):
            return self.sem(SEM_KV + 5 * (g % 2) + slot)

        def kv(self, priority, g, slot, kv, b0, nb, r0, nr, sem=None):
            def start():
                if slot == GQA_SLOT:
                    src = (ka_hbm, va_hbm)[kv].at[pl.ds(b0, nb), g, pl.ds(r0, nr)]
                else:
                    src = (kb_hbm, vb_hbm)[kv].at[pl.ds(b0, nb), 4 * g + slot, pl.ds(r0, nr)]
                dst = kv_buf.at[slot, kv, pl.ds(b0, nb), pl.ds(r0, nr)]
                s = self.kv_sem(g, slot) if sem is None else self.sem(sem)
                pltpu.make_async_copy(src, dst, s).start(priority=priority)
            return start

        def bulk(self, g, slot, first, lo, hi):
            return [self.kv(BULK, g, slot, kv, b0, min(4, BATCH - b0), r0, 64)
                    for r0 in range(lo, hi, 64) for kv in (0, 1) for b0 in (first, first + 4)]

        def batch0(self, g, slot):
            return [self.kv(FILL, g, slot, kv, 0, 1, r0 + r, 32)
                    for r0 in range(0, SK, 64) for kv in (0, 1) for r in (0, 32)]

        def weights(self, g, which, priority=FILL, nr=8):
            def piece(r0):
                def start():
                    base = g * GROUP_W if isinstance(g, int) else pl.multiple_of(g * GROUP_W, GROUP_W)
                    if which < 2:
                        src = (wqa_hbm, wqb_hbm)[which].at[pl.ds(r0, nr), pl.ds(base, GROUP_W)]
                    else:
                        src = (woa_hbm, wob_hbm)[which - 2].at[pl.ds(base + r0, nr)]
                    dst = w_buf.at[g % 2, which, pl.ds(r0, nr)]
                    pltpu.make_async_copy(src, dst, self.sem(SEM_W + g)).start(priority=priority)
                return start
            if which < 2:
                return [piece(64 * i + r0) for r0 in range(0, 64, nr) for i in range(8)]
            return [piece(r0) for r0 in range(0, GROUP_W, nr)]

        def x(self):
            def piece(br, r0):
                def start():
                    src = (xa_hbm, xb_hbm)[br].at[pl.ds(r0, 16)]
                    pltpu.make_async_copy(src, x_buf.at[br, pl.ds(r0, 16)], self.sem(SEM_X)).start(priority=BULK)
                return start
            return [piece(br, r0) for r0 in range(0, M, 16) for br in (0, 1)]

        def window(self, nxt, after, weights=None):
            fill = self.batch0(*after[:2]) if weights is None else self.weights(*weights)
            bulk = self.bulk(*nxt, AHEAD_ROWS, SK) + self.bulk(*after, 0, AHEAD_ROWS)
            return _interleave(bulk, fill)

        def last_head(self):
            g, fill = GROUPS - 1, []
            bulk = self.bulk(g, 2, 1, AHEAD_ROWS, SK)
            parts = [(b0, nb, (0, 1)) for b0, nb in LAST_PARTS[:-1]]
            parts += [(*LAST_PARTS[-1], (0,)), (*LAST_PARTS[-1], (1,))]
            for i, (b0, nb, kvs) in enumerate(parts):
                def sem(r0):
                    return SEM_LAST + i + (1 if kvs == (1,) and r0 >= LAST_V_CUT else 0)
                bulk += [self.kv(BULK, g, 3, kv, b0, nb, r0, 64, sem(r0))
                         for r0 in range(LAST_FILL_ROWS, SK, 64) for kv in kvs]
                fill += [self.kv(FILL, g, 3, kv, b, 1, r0, 32, sem(r0))
                         for r0 in range(0, LAST_FILL_ROWS, 32) for b in range(b0, b0 + nb) for kv in kvs]
            return _interleave(bulk, fill)

    def wait_filled(ref, sem):
        pltpu.make_async_copy(ref, ref, sem).wait()

    def gqa_phase(copies, g, starts):
        live = {}

        def q_proj(pair):
            q = (_dot(x_buf[0, 2 * SQ * pair:2 * SQ * (pair + 1), :], w_buf[g % 2, 0]) * Q_SCALE).astype(bf16)
            for u in range(2):
                live["q", 2 * pair + u] = jnp.concatenate(
                    [q[u * SQ:(u + 1) * SQ, i * DH:(i + 1) * DH] for i in range(4)], axis=0)

        def qk(b):
            live["s", b] = _scores(live.pop(("q", b)), kv_buf[GQA_SLOT, 0, b])

        def pv(b):
            p, denom = _exp_and_sum(live.pop(("s", b)))
            live["o", b] = _normalize(_dot(p, kv_buf[GQA_SLOT, 1, b]), denom)

        def o_proj(pair):
            o = [live.pop(("o", 2 * pair + u)) for u in range(2)]
            o = jnp.concatenate(
                [jnp.concatenate([ou[i * SQ:(i + 1) * SQ] for i in range(4)], axis=1) for ou in o], axis=0)
            acc_a[2 * SQ * pair:2 * SQ * (pair + 1), :] += _dot(o, w_buf[g % 2, 2])

        stages = [(384, lambda: q_proj(0))]
        for b in range(BATCH + 1):
            if b % 2 == 1 and b + 1 < BATCH:
                stages.append((384, lambda b=b: q_proj((b + 1) // 2)))
            if b < BATCH:
                stages.append((400, lambda b=b: qk(b)))
            if b >= 1:
                stages.append((400, lambda b=b: pv(b - 1)))
            if b % 2 == 1 and b >= 3:
                stages.append((384, lambda b=b: o_proj((b - 3) // 2)))
        stages.append((384, lambda: o_proj(3)))

        wait_filled(w_buf.at[g % 2], copies.sem(SEM_W + g))
        wait_filled(kv_buf.at[GQA_SLOT], copies.kv_sem(g, GQA_SLOT))
        _run(stages, starts, 8)

    def mha_q(g, j):
        return (_dot(x_buf[1], w_buf[g % 2, 1, :, j * DH:(j + 1) * DH]) * Q_SCALE).astype(bf16)

    def mha_y(g, j, b0, o):
        w = w_buf[g % 2, 3, j * DH:(j + 1) * DH, :]
        return _dot(jnp.concatenate(o, axis=0), w) + acc_b[b0 * SQ:(b0 + len(o)) * SQ, :]

    def mha_phase(copies, g, j, starts):
        live = {}

        def q_proj():
            live["q"] = mha_q(g, j)

        def qk(b):
            live["s", b] = _scores(live["q"][b * SQ:(b + 1) * SQ], kv_buf[j, 0, b])

        def pv(b):
            p, denom = _exp_and_sum(live.pop(("s", b)))
            live["o", b] = _normalize(_dot(p, kv_buf[j, 1, b]), denom)

        def o_proj(b0):
            acc_b[b0 * SQ:(b0 + 4) * SQ, :] = mha_y(g, j, b0, [live.pop(("o", b)) for b in range(b0, b0 + 4)])

        stages = [(384, q_proj)]
        for b in range(BATCH + 2):
            if b < BATCH:
                stages.append((128, lambda b=b: qk(b)))
            if b >= 2:
                stages.append((110, lambda b=b: pv(b - 2)))
            if b == BATCH - 1:
                stages.append((192, lambda: o_proj(0)))
        stages.append((192, lambda: o_proj(4)))

        wait_filled(kv_buf.at[j], copies.kv_sem(g, j))
        _run(stages, starts, 4)

    def prologue(copies):
        small = _interleave(copies.x(), copies.weights(0, 2, BULK, 16), copies.weights(0, 3, BULK, 16))
        starts = (small[:LEAD] + _interleave(small[LEAD:], copies.weights(0, 1))
                  + _interleave(copies.bulk(0, GQA_SLOT, 0, 0, SK), copies.weights(0, 0))
                  + _interleave(copies.bulk(0, 0, 1, 0, AHEAD_ROWS), copies.batch0(0, 0)))
        for start in starts:
            start()
        acc_a[...] = jnp.zeros_like(acc_a)
        acc_b[...] = jnp.zeros_like(acc_b)
        wait_filled(x_buf, copies.sem(SEM_X))

    def first_two_phases(copies, g, window_a, window_0):
        early = len(window_0) // 4
        gqa_phase(copies, g, window_a + window_0[:early])
        mha_phase(copies, g, 0, window_0[early:])

    def group(copies, g):
        phases = [(g, 0, 1), (g, 1, 0), (g, 2, 0), (g, 3, 0), (g + 1, GQA_SLOT, 0), (g + 1, 0, 1)]
        windows = [copies.window(phases[i], phases[i + 1], (g + 1, i) if i < 4 else None) for i in range(5)]
        first_two_phases(copies, g, windows[0], windows[1])
        for j in range(1, 4):
            mha_phase(copies, g, j, windows[j + 1])

    def last_group(copies):
        g = GROUPS - 1
        phases = [(g, j, 1) for j in range(3)]
        first_two_phases(copies, g, copies.window(phases[0], phases[1]), copies.window(phases[1], phases[2]))
        ya_buf[...] = acc_a[...].astype(bf16)
        starts = copies.last_head()
        cut = len(starts) * AHEAD_ROWS // SK
        mha_phase(copies, g, 1, starts[:cut])
        mha_phase(copies, g, 2, starts[cut:])

        q = mha_q(g, 3)

        def probs(b0, nb):
            s = [_scores(q[b * SQ:(b + 1) * SQ], kv_buf[3, 0, b]) for b in range(b0, b0 + nb)]
            return [_exp_and_sum(sb) for sb in s]

        def finish(b0, p, y_buf):
            o = [_normalize(_dot(pb, kv_buf[3, 1, b0 + i]), denom) for i, (pb, denom) in enumerate(p)]
            y_buf[...] = mha_y(g, 3, b0, o).astype(bf16)

        writes = [pltpu.make_async_copy(ya_buf, out_hbm.at[:, pl.ds(0, D)], out_sems.at[0])]
        for i, (b0, nb) in enumerate(LAST_PARTS):
            dst = out_hbm.at[pl.ds(b0 * SQ, nb * SQ), pl.ds(D, D)]
            writes.append(pltpu.make_async_copy(yb_bufs[i], dst, out_sems.at[1 + i]))

        for i, (b0, nb) in enumerate(LAST_PARTS[:-1]):
            wait_filled(kv_buf.at[3, :, pl.ds(b0, nb)], copies.sem(SEM_LAST + i))
            finish(b0, probs(b0, nb), yb_bufs[i])
        b0, nb = LAST_PARTS[-1]
        sem = SEM_LAST + len(LAST_PARTS) - 1
        wait_filled(kv_buf.at[3, 0, pl.ds(b0, nb)], copies.sem(sem))
        wait_filled(kv_buf.at[3, 1, pl.ds(b0, nb), pl.ds(0, LAST_V_CUT)], copies.sem(sem + 1))
        for write in writes[:-1]:
            write.start()
        p = probs(b0, nb)
        wait_filled(kv_buf.at[3, 1, pl.ds(b0, nb), pl.ds(LAST_V_CUT, SK - LAST_V_CUT)], copies.sem(sem + 2))
        finish(b0, p, yb_bufs[-1])
        writes[-1].start()
        for write in writes:
            write.wait()

    def body(g, carry):
        @pl.when(g == 0)
        def _():
            prologue(Copies(g))

        @pl.when(g < GROUPS - 1)
        def _():
            group(Copies(0), g)

        @pl.when(g == GROUPS - 1)
        def _():
            last_group(Copies(g - (GROUPS - 1)))

        return carry

    jax.lax.fori_loop(0, GROUPS, body, 0)


@jax.jit
def pallas_concat_heads__gqa_block_cached__mha_block_cached__near_ridge_kernel(
    A_x: jax.Array,
    A_k_cache: jax.Array,
    A_v_cache: jax.Array,
    A_wq: jax.Array,
    A_wo: jax.Array,
    B_x: jax.Array,
    B_k_cache: jax.Array,
    B_v_cache: jax.Array,
    B_wq: jax.Array,
    B_wo: jax.Array,
):
    out = pl.pallas_call(
        _kernel,
        in_specs=[pl.BlockSpec(memory_space=pltpu.HBM)] * 10,
        out_specs=pl.BlockSpec(memory_space=pltpu.HBM),
        out_shape=jax.ShapeDtypeStruct((M, 2 * D), bf16),
        scratch_shapes=[
            pltpu.VMEM((5, 2, BATCH, SK, DH), bf16),
            pltpu.VMEM((2, M, D), bf16),
            pltpu.VMEM((2, 4, GROUP_W, D), bf16),
            pltpu.VMEM((M, D), f32),
            pltpu.VMEM((M, D), f32),
            pltpu.SemaphoreType.DMA((NUM_SEMS,)),
            pltpu.SemaphoreType.DMA((1 + len(LAST_PARTS),)),
            pltpu.VMEM((M, D), bf16),
            *[pltpu.VMEM((nb * SQ, D), bf16) for _, nb in LAST_PARTS],
        ],
        compiler_params=pltpu.CompilerParams(
            vmem_limit_bytes=64 * 2 ** 20,
            disable_bounds_checks=True,
            disable_semaphore_checks=True,
        ),
        name="gqa_mha_cached_blocks",
    )(A_x.reshape(M, D), A_k_cache, A_v_cache, A_wq, A_wo,
      B_x.reshape(M, D), B_k_cache, B_v_cache, B_wq, B_wo)
    return out.reshape(BATCH, SQ, 2 * D)
```

```python
import math

import jax
import jax.numpy as jnp
import jax.experimental.pallas as pl
import jax.experimental.pallas.tpu as pltpu

BATCH, SQ, D = 8, 48, 512
SK, DH = 1024, 128
GROUPS = 8
GROUP_W = 4 * DH
M = BATCH * SQ
Q_SCALE = DH ** -0.5 * math.log2(math.e)

GQA_SLOT = 4
BULK, FILL = 1, 0
AHEAD_ROWS = 768
LAST_FILL_ROWS = 128
LAST_PARTS = ((0, 4), (4, 2), (6, 2))
LAST_V_CUT = 448

SEM_KV, SEM_W, SEM_X, SEM_LAST, NUM_SEMS = 0, 10, 18, 19, 24

f32, bf16 = jnp.float32, jnp.bfloat16


def _dot(a, b):
    return jnp.dot(a, b, preferred_element_type=f32)


def _scores(q, k):
    return jax.lax.dot_general(q, k, (((1,), (1,)), ((), ())), preferred_element_type=f32)


def _exp_and_sum(s):
    p = jnp.exp2(s - jnp.max(s, axis=-1, keepdims=True))
    return p.astype(bf16), jnp.sum(p, axis=-1, keepdims=True)


def _normalize(o, denom):
    return (o * (1.0 / denom)).astype(bf16)


def _interleave(*seqs):
    keyed = [((i + 0.5) / len(seq), w, i) for w, seq in enumerate(seqs) for i in range(len(seq))]
    return [seqs[w][i] for _, w, i in sorted(keyed)]


def _run(stages, starts, points):
    total = sum(cost for cost, _ in stages)
    spent, started, point = 0, 0, 0
    for cost, stage in stages:
        while point < points and spent * points >= total * point:
            point += 1
        upto = len(starts) * point // points
        for start in starts[started:upto]:
            start()
        started = upto
        stage()
        spent += cost
    for start in starts[started:]:
        start()


def _kernel(xa_hbm, ka_hbm, va_hbm, wqa_hbm, woa_hbm, xb_hbm, kb_hbm, vb_hbm, wqb_hbm, wob_hbm, out_hbm,
            kv_buf, x_buf, w_buf, acc_a, acc_b, sems, out_sems, ya_buf, *yb_bufs):

    class Copies:
        def __init__(self, zero):
            self.zero = zero

        def sem(self, i):
            return sems.at[i + self.zero]

        def kv_sem(self, g, slot):
            return self.sem(SEM_KV + 5 * (g % 2) + slot)

        def kv(self, priority, g, slot, kv, b0, nb, r0, nr, sem=None):
            def start():
                if slot == GQA_SLOT:
                    src = (ka_hbm, va_hbm)[kv].at[pl.ds(b0, nb), g, pl.ds(r0, nr)]
                else:
                    src = (kb_hbm, vb_hbm)[kv].at[pl.ds(b0, nb), 4 * g + slot, pl.ds(r0, nr)]
                dst = kv_buf.at[slot, kv, pl.ds(b0, nb), pl.ds(r0, nr)]
                s = self.kv_sem(g, slot) if sem is None else self.sem(sem)
                pltpu.make_async_copy(src, dst, s).start(priority=priority)
            return start

        def bulk(self, g, slot, first, lo, hi):
            return [self.kv(BULK, g, slot, kv, b0, min(4, BATCH - b0), r0, 64)
                    for r0 in range(lo, hi, 64) for kv in (0, 1) for b0 in (first, first + 4)]

        def batch0(self, g, slot):
            return [self.kv(FILL, g, slot, kv, 0, 1, r0 + r, 32)
                    for r0 in range(0, SK, 64) for kv in (0, 1) for r in (0, 32)]

        def weights(self, g, which, priority=FILL, nr=8):
            def piece(r0):
                def start():
                    base = g * GROUP_W if isinstance(g, int) else pl.multiple_of(g * GROUP_W, GROUP_W)
                    if which < 2:
                        src = (wqa_hbm, wqb_hbm)[which].at[pl.ds(r0, nr), pl.ds(base, GROUP_W)]
                    else:
                        src = (woa_hbm, wob_hbm)[which - 2].at[pl.ds(base + r0, nr)]
                    dst = w_buf.at[g % 2, which, pl.ds(r0, nr)]
                    pltpu.make_async_copy(src, dst, self.sem(SEM_W + g)).start(priority=priority)
                return start
            if which < 2:
                return [piece(64 * i + r0) for r0 in range(0, 64, nr) for i in (0, 4, 1, 5, 2, 6, 3, 7)]
            return [piece(r0) for r0 in range(0, GROUP_W, nr)]

        def x(self):
            def piece(br, r0):
                def start():
                    src = (xa_hbm, xb_hbm)[br].at[pl.ds(r0, 16)]
                    pltpu.make_async_copy(src, x_buf.at[br, pl.ds(r0, 16)], self.sem(SEM_X)).start(priority=BULK)
                return start
            return [piece(br, r0) for r0 in range(0, M, 16) for br in (0, 1)]

        def window(self, nxt, after, weights=None):
            fill = self.batch0(*after[:2]) if weights is None else self.weights(*weights)
            bulk = self.bulk(*nxt, AHEAD_ROWS, SK) + self.bulk(*after, 0, AHEAD_ROWS)
            return _interleave(bulk, fill)

        def last_head(self):
            g, fill = GROUPS - 1, []
            bulk = self.bulk(g, 2, 1, AHEAD_ROWS, SK)
            parts = [(b0, nb, (0, 1)) for b0, nb in LAST_PARTS[:-1]]
            parts += [(*LAST_PARTS[-1], (0,)), (*LAST_PARTS[-1], (1,))]
            for i, (b0, nb, kvs) in enumerate(parts):
                def sem(r0):
                    return SEM_LAST + i + (1 if kvs == (1,) and r0 >= LAST_V_CUT else 0)
                bulk += [self.kv(BULK, g, 3, kv, b0, nb, r0, 64, sem(r0))
                         for r0 in range(LAST_FILL_ROWS, SK, 64) for kv in kvs]
                fill += [self.kv(FILL, g, 3, kv, b, 1, r0, 32, sem(r0))
                         for r0 in range(0, LAST_FILL_ROWS, 32) for b in range(b0, b0 + nb) for kv in kvs]
            return _interleave(bulk, fill)

    def wait_filled(ref, sem):
        pltpu.make_async_copy(ref, ref, sem).wait()

    def gqa_phase(copies, g, starts):
        live = {}

        def q_proj(pair):
            q = (_dot(x_buf[0, 2 * SQ * pair:2 * SQ * (pair + 1), :], w_buf[g % 2, 0]) * Q_SCALE).astype(bf16)
            for u in range(2):
                live["q", 2 * pair + u] = jnp.concatenate(
                    [q[u * SQ:(u + 1) * SQ, i * DH:(i + 1) * DH] for i in range(4)], axis=0)

        def qk(b):
            live["s", b] = _scores(live.pop(("q", b)), kv_buf[GQA_SLOT, 0, b])

        def pv(b):
            p, denom = _exp_and_sum(live.pop(("s", b)))
            live["o", b] = _normalize(_dot(p, kv_buf[GQA_SLOT, 1, b]), denom)

        def o_proj(pair):
            o = [live.pop(("o", 2 * pair + u)) for u in range(2)]
            o = jnp.concatenate(
                [jnp.concatenate([ou[i * SQ:(i + 1) * SQ] for i in range(4)], axis=1) for ou in o], axis=0)
            acc_a[2 * SQ * pair:2 * SQ * (pair + 1), :] += _dot(o, w_buf[g % 2, 2])

        stages = [(384, lambda: q_proj(0))]
        for b in range(BATCH + 1):
            if b % 2 == 1 and b + 1 < BATCH:
                stages.append((384, lambda b=b: q_proj((b + 1) // 2)))
            if b < BATCH:
                stages.append((400, lambda b=b: qk(b)))
            if b >= 1:
                stages.append((400, lambda b=b: pv(b - 1)))
            if b % 2 == 1 and b >= 3:
                stages.append((384, lambda b=b: o_proj((b - 3) // 2)))
        stages.append((384, lambda: o_proj(3)))

        wait_filled(w_buf.at[g % 2], copies.sem(SEM_W + g))
        wait_filled(kv_buf.at[GQA_SLOT], copies.kv_sem(g, GQA_SLOT))
        _run(stages, starts, 8)

    def mha_q(g, j):
        return (_dot(x_buf[1], w_buf[g % 2, 1, :, j * DH:(j + 1) * DH]) * Q_SCALE).astype(bf16)

    def mha_y(g, j, b0, o):
        w = w_buf[g % 2, 3, j * DH:(j + 1) * DH, :]
        return _dot(jnp.concatenate(o, axis=0), w) + acc_b[b0 * SQ:(b0 + len(o)) * SQ, :]

    def mha_phase(copies, g, j, starts):
        live = {}

        def q_proj():
            live["q"] = mha_q(g, j)

        def qk(b):
            live["s", b] = _scores(live["q"][b * SQ:(b + 1) * SQ], kv_buf[j, 0, b])

        def pv(b):
            p, denom = _exp_and_sum(live.pop(("s", b)))
            live["o", b] = _normalize(_dot(p, kv_buf[j, 1, b]), denom)

        def o_proj(b0):
            acc_b[b0 * SQ:(b0 + 4) * SQ, :] = mha_y(g, j, b0, [live.pop(("o", b)) for b in range(b0, b0 + 4)])

        stages = [(384, q_proj)]
        for b in range(BATCH + 2):
            if b < BATCH:
                stages.append((128, lambda b=b: qk(b)))
            if b >= 2:
                stages.append((110, lambda b=b: pv(b - 2)))
            if b == BATCH - 1:
                stages.append((192, lambda: o_proj(0)))
        stages.append((192, lambda: o_proj(4)))

        wait_filled(kv_buf.at[j], copies.kv_sem(g, j))
        _run(stages, starts, 4)

    def prologue(copies):
        small = copies.x() + _interleave(copies.weights(0, 2, BULK, 16), copies.weights(0, 3, BULK, 16))
        starts = (_interleave(small, copies.weights(0, 1))
                  + _interleave(copies.bulk(0, GQA_SLOT, 0, 0, SK), copies.weights(0, 0))
                  + _interleave(copies.bulk(0, 0, 1, 0, AHEAD_ROWS), copies.batch0(0, 0)))
        for start in starts:
            start()
        acc_a[...] = jnp.zeros_like(acc_a)
        acc_b[...] = jnp.zeros_like(acc_b)
        wait_filled(x_buf, copies.sem(SEM_X))

    def first_two_phases(copies, g, window_a, window_0):
        early = len(window_0) // 4
        gqa_phase(copies, g, window_a + window_0[:early])
        mha_phase(copies, g, 0, window_0[early:])

    def group(copies, g):
        phases = [(g, 0, 1), (g, 1, 0), (g, 2, 0), (g, 3, 0), (g + 1, GQA_SLOT, 0), (g + 1, 0, 1)]
        windows = [copies.window(phases[i], phases[i + 1], (g + 1, i) if i < 4 else None) for i in range(5)]
        first_two_phases(copies, g, windows[0], windows[1])
        for j in range(1, 4):
            mha_phase(copies, g, j, windows[j + 1])

    def last_group(copies):
        g = GROUPS - 1
        phases = [(g, j, 1) for j in range(3)]
        first_two_phases(copies, g, copies.window(phases[0], phases[1]), copies.window(phases[1], phases[2]))
        ya_buf[...] = acc_a[...].astype(bf16)
        starts = copies.last_head()
        cut = len(starts) * AHEAD_ROWS // SK
        mha_phase(copies, g, 1, starts[:cut])
        mha_phase(copies, g, 2, starts[cut:])

        q = mha_q(g, 3)

        def probs(b0, nb):
            s = [_scores(q[b * SQ:(b + 1) * SQ], kv_buf[3, 0, b]) for b in range(b0, b0 + nb)]
            return [_exp_and_sum(sb) for sb in s]

        def finish(b0, p, y_buf):
            o = [_normalize(_dot(pb, kv_buf[3, 1, b0 + i]), denom) for i, (pb, denom) in enumerate(p)]
            y_buf[...] = mha_y(g, 3, b0, o).astype(bf16)

        writes = [pltpu.make_async_copy(ya_buf, out_hbm.at[:, pl.ds(0, D)], out_sems.at[0])]
        for i, (b0, nb) in enumerate(LAST_PARTS):
            dst = out_hbm.at[pl.ds(b0 * SQ, nb * SQ), pl.ds(D, D)]
            writes.append(pltpu.make_async_copy(yb_bufs[i], dst, out_sems.at[1 + i]))

        for i, (b0, nb) in enumerate(LAST_PARTS[:-1]):
            wait_filled(kv_buf.at[3, :, pl.ds(b0, nb)], copies.sem(SEM_LAST + i))
            finish(b0, probs(b0, nb), yb_bufs[i])
        b0, nb = LAST_PARTS[-1]
        sem = SEM_LAST + len(LAST_PARTS) - 1
        wait_filled(kv_buf.at[3, 0, pl.ds(b0, nb)], copies.sem(sem))
        wait_filled(kv_buf.at[3, 1, pl.ds(b0, nb), pl.ds(0, LAST_V_CUT)], copies.sem(sem + 1))
        for write in writes[:-1]:
            write.start()
        p = probs(b0, nb)
        wait_filled(kv_buf.at[3, 1, pl.ds(b0, nb), pl.ds(LAST_V_CUT, SK - LAST_V_CUT)], copies.sem(sem + 2))
        finish(b0, p, yb_bufs[-1])
        writes[-1].start()
        for write in writes:
            write.wait()

    def body(g, carry):
        @pl.when(g == 0)
        def _():
            prologue(Copies(g))

        @pl.when(g < GROUPS - 1)
        def _():
            group(Copies(0), g)

        @pl.when(g == GROUPS - 1)
        def _():
            last_group(Copies(g - (GROUPS - 1)))

        return carry

    jax.lax.fori_loop(0, GROUPS, body, 0)


@jax.jit
def pallas_concat_heads__gqa_block_cached__mha_block_cached__near_ridge_kernel(
    A_x: jax.Array,
    A_k_cache: jax.Array,
    A_v_cache: jax.Array,
    A_wq: jax.Array,
    A_wo: jax.Array,
    B_x: jax.Array,
    B_k_cache: jax.Array,
    B_v_cache: jax.Array,
    B_wq: jax.Array,
    B_wo: jax.Array,
):
    out = pl.pallas_call(
        _kernel,
        in_specs=[pl.BlockSpec(memory_space=pltpu.HBM)] * 10,
        out_specs=pl.BlockSpec(memory_space=pltpu.HBM),
        out_shape=jax.ShapeDtypeStruct((M, 2 * D), bf16),
        scratch_shapes=[
            pltpu.VMEM((5, 2, BATCH, SK, DH), bf16),
            pltpu.VMEM((2, M, D), bf16),
            pltpu.VMEM((2, 4, GROUP_W, D), bf16),
            pltpu.VMEM((M, D), f32),
            pltpu.VMEM((M, D), f32),
            pltpu.SemaphoreType.DMA((NUM_SEMS,)),
            pltpu.SemaphoreType.DMA((1 + len(LAST_PARTS),)),
            pltpu.VMEM((M, D), bf16),
            *[pltpu.VMEM((nb * SQ, D), bf16) for _, nb in LAST_PARTS],
        ],
        compiler_params=pltpu.CompilerParams(
            vmem_limit_bytes=64 * 2 ** 20,
            disable_bounds_checks=True,
            disable_semaphore_checks=True,
        ),
        name="gqa_mha_cached_blocks",
    )(A_x.reshape(M, D), A_k_cache, A_v_cache, A_wq, A_wo,
      B_x.reshape(M, D), B_k_cache, B_v_cache, B_wq, B_wo)
    return out.reshape(BATCH, SQ, 2 * D)
```
